```python
import jax
import jax.numpy as jnp

def _softmax(x, axis=-1):
    return jax.nn.softmax(x, axis=axis)

def _gelu(x):
    return jax.nn.gelu(x, approximate=True)

def _silu(x):
    return jax.nn.silu(x)

def _sigmoid(x):
    return jax.nn.sigmoid(x)

def _layernorm(x, axis=-1, eps=1e-05):
    m = jnp.mean(x, axis=axis, keepdims=True)
    v = jnp.var(x, axis=axis, keepdims=True)
    return (x - m) / jnp.sqrt(v + eps)

def _scatter_add(tgt, idx, src, axis=0):
    return tgt.at[idx].add(src)

def _segment_sum(src, seg, n):
    return jax.ops.segment_sum(src, seg, n)

class _Rng:

    def __init__(self, key):
        self._k = key

    def _next(self):
        self._k, sub = jax.random.split(self._k)
        return sub

    def normal(self, shape):
        return jax.random.normal(self._next(), shape, dtype=jnp.bfloat16)

    def randint(self, lo, hi, shape):
        return jax.random.randint(self._next(), shape, lo, hi, dtype=jnp.int32)

    def uniform(self, shape, lo=0.0, hi=1.0):
        return jax.random.uniform(self._next(), shape, jnp.bfloat16, lo, hi)

    def permutation(self, n):
        return jax.random.permutation(self._next(), n)
kernel_name = 'adaLN_cond__ssm_conv_h3__glu_gated_swiglu__prompt'

def setup_inputs():
    _rng = _Rng(jax.random.key(int.from_bytes(__import__("os").urandom(4), "little")))
    _w = lambda a: (lambda t: t.astype(jnp.bfloat16) if jnp.issubdtype(t.dtype, jnp.floating) else t)(jnp.asarray(a))

    def _A_setup():
        B, S, D = (1, 2048, 640)
        ks = 4
        return {'q': _w((lambda *s: _rng.normal(s) * 0.05)(B, S, D)), 'k': _w((lambda *s: _rng.normal(s) * 0.05)(B, S, D)), 'v': _w((lambda *s: _rng.normal(s) * 0.05)(B, S, D)), 'shift_k': _w((lambda *s: _rng.normal(s) * 0.05)(D, ks) * 0.5), 'ssm_k': _w((lambda *s: _rng.normal(s) * 0.05)(D, S) * (1.0 / S ** 0.5)), 'ssm_D': _w((lambda *s: _rng.normal(s) * 0.05)(D))}
    _A_in = _A_setup()

    def _B_setup():
        B, S, D, F = (1, 2048, 640, 1536)
        return {'x': _w((lambda *s: _rng.normal(s) * 0.05)(B, S, D)), 'w1': _w((lambda *s: _rng.normal(s) * 0.05)(D, F) * (2.0 / D) ** 0.5), 'w3': _w((lambda *s: _rng.normal(s) * 0.05)(D, F) * (2.0 / D) ** 0.5), 'w2': _w((lambda *s: _rng.normal(s) * 0.05)(F, D) * (2.0 / F) ** 0.5)}
    _B_in = _B_setup()
    return {'A_q': _A_in['q'], 'A_k': _A_in['k'], 'A_v': _A_in['v'], 'A_shift_k': _A_in['shift_k'], 'A_ssm_k': _A_in['ssm_k'], 'A_ssm_D': _A_in['ssm_D'], 'B_x': _B_in['x'], 'B_w1': _B_in['w1'], 'B_w3': _B_in['w3'], 'B_w2': _B_in['w2'], 'c': _w((lambda *s: _rng.normal(s) * 0.05)(1, 640)), 'w_mod': _w((lambda *s: _rng.normal(s) * 0.05)(640, 6 * 640) * 640 ** (-0.5))}

def reference(A_q, A_k, A_v, A_shift_k, A_ssm_k, A_ssm_D, B_x, B_w1, B_w3, B_w2, c, w_mod):

    def _A_ref(q, k, v, shift_k, ssm_k, ssm_D):
        B, S, D = q.shape
        ks = shift_k.shape[-1]
        k_pad = jnp.pad(k, ((0, 0), (ks - 1, 0), (0, 0)))
        k_shift = jnp.zeros_like(k)
        for t in range(ks):
            k_shift = k_shift + k_pad[:, t:t + S, :] * shift_k[:, ks - 1 - t][None, None, :]
        kv = k_shift * v
        L = 2 * S
        kv_pad = jnp.pad(kv, ((0, 0), (0, S), (0, 0)))
        kf_pad = jnp.pad(ssm_k, ((0, 0), (0, S)))
        kv_f = (lambda x, axes=(-2, -1): jnp.fft.rfft2(x.astype(jnp.float32), axes=axes))(kv_pad[:, None, :, :], axes=(1, 2))
        kf_f = (lambda x, axes=(-2, -1): jnp.fft.rfft2(x.astype(jnp.float32), axes=axes))(kf_pad[:, None, :], axes=(1, 2))
        kf_f = (lambda x, *d: x.transpose(*d))(kf_f, 1, 2, 0)
        y_f = kv_f * kf_f[None, :, :, :]
        y = (lambda x, s, axes=(-2, -1): jnp.fft.irfft2(x, s=s, axes=axes).astype(jnp.bfloat16))(y_f, (1, L), axes=(1, 2))[:, 0, :S, :]
        y = y + kv * ssm_D[None, None, :]
        return q * y

    def _B_ref(x, w1, w3, w2):
        gate = jnp.einsum('bsd,df->bsf', x, w1)
        up = jnp.einsum('bsd,df->bsf', x, w3)
        h = _silu(gate) * up
        out = jnp.einsum('bsf,fd->bsd', h, w2)
        return out
    x = A_q
    mod = (_silu(c) @ w_mod).reshape(c.shape[0], 6, 1, -1)
    sa, ca, ga, sb, cb, gb = (mod[:, 0].copy(), mod[:, 1].copy(), mod[:, 2].copy(), mod[:, 3].copy(), mod[:, 4].copy(), mod[:, 5].copy())
    h = _layernorm(x, axis=-1) * (1 + ca) + sa
    x = x + ga * _A_ref(h, A_k, A_v, A_shift_k, A_ssm_k, A_ssm_D)
    h = _layernorm(x, axis=-1) * (1 + cb) + sb
    x = x + gb * _B_ref(h, B_w1, B_w3, B_w2)
    return x
```

```python
import numpy as np
import jax
import jax.numpy as jnp
import jax.experimental.pallas as pl
import jax.experimental.pallas.tpu as pltpu

S, D, FF = 2048, 640, 1536
B = 128
NB = S // B
N2 = 2 * B
EPS = 1e-5

CFG = dict(TM=256, FC=256, MR=16, MC=256, ER=32, mode='all', inter=True)

f32 = jnp.float32
bf16 = jnp.bfloat16


def _dft_matrices():
    f = np.concatenate([np.arange(0, B, 2), np.arange(1, B, 2)])
    ang = 2.0 * np.pi * np.outer(f + 0.5, np.arange(B)) / N2
    fwd = np.concatenate([np.cos(ang), -np.sin(ang)], axis=0)
    inv = fwd.T / B
    return fwd.astype(jnp.bfloat16), np.ascontiguousarray(inv).astype(jnp.bfloat16)


def _interleave(*tasks):
    tasks = [t for t in tasks if t]
    keyed = []
    for ti, t in enumerate(tasks):
        for i, th in enumerate(t):
            keyed.append(((i + 0.5) / len(t), ti, i, th))
    keyed.sort(key=lambda e: e[:3])
    for e in keyed:
        e[3]()


def _kernel(q_hbm, k_hbm, v_hbm, shk_hbm, ssmk_hbm, dd_hbm, w1_hbm, w3_hbm, w2_hbm, c_hbm,
            wmod_hbm, fwd_hbm, inv_hbm, out_hbm,
            q_v, k_v, v_v, shk_v, ssmk_v, dd_v, w1_v, w3_v, w2_v, c_v, wmod_v, fwd_v, inv_v,
            xs, hs, hraw, kf, kv32, zb, x1, hb, act, ob, mod_v, sems):
    TM, FC, MR, MC, ER = CFG['TM'], CFG['FC'], CFG['MR'], CFG['MC'], CFG['ER']
    mode = CFG['mode']
    NS = S // TM
    BPS = TM // B
    NF = FF // FC
    do_conv = mode in ('all', 'conv')
    do_ffn = mode in ('all', 'ffn')

    nsem = [0]
    def copy(src, dst):
        cp = pltpu.make_async_copy(src, dst, sems.at[nsem[0]])
        nsem[0] += 1
        return cp

    def rows(j):
        return pl.ds(j * TM, TM)

    cp_small = [copy(c_hbm, c_v), copy(shk_hbm, shk_v), copy(dd_hbm, dd_v),
                copy(fwd_hbm, fwd_v), copy(inv_hbm, inv_v)]
    cp_k = [copy(k_hbm.at[rows(j)], k_v.at[rows(j)]) for j in range(NS)]
    cp_v = [copy(v_hbm.at[rows(j)], v_v.at[rows(j)]) for j in range(NS)]
    cp_s = [copy(ssmk_hbm.at[:, rows(j)], ssmk_v.at[:, rows(j)]) for j in range(NS)]
    cp_q = [copy(q_hbm.at[rows(j)], q_v.at[rows(j)]) for j in range(NS)]
    cp_m = [copy(wmod_hbm.at[:, pl.ds(i * D, D)], wmod_v.at[:, pl.ds(i * D, D)]) for i in range(6)]
    cp_w1 = [copy(w1_hbm.at[:, pl.ds(i * FC, FC)], w1_v.at[:, pl.ds(i * FC, FC)]) for i in range(NF)]
    cp_w3 = [copy(w3_hbm.at[:, pl.ds(i * FC, FC)], w3_v.at[:, pl.ds(i * FC, FC)]) for i in range(NF)]
    cp_w2 = copy(w2_hbm, w2_v)
    cp_o = [copy(ob.at[rows(j)], out_hbm.at[rows(j)]) for j in range(NS)]

    for cp in cp_small + [cp_k[0], cp_v[0], cp_s[0], cp_q[0]] + cp_m[:5]:
        cp.start()
    for i in range(NF):
        cp_w1[i].start()
        cp_w3[i].start()
    for cp in [cp_k[1], cp_v[1], cp_s[1], cp_q[1], cp_w2, cp_m[5]]:
        cp.start()
    for j in range(2, NS):
        for cp in (cp_k[j], cp_v[j], cp_s[j], cp_q[j]):
            cp.start()

    for cp in cp_small:
        cp.wait()

    def stage_a(j):
        th = []
        def load():
            cp_k[j].wait(); cp_v[j].wait(); cp_s[j].wait()
            if j == 0:
                kf[0:8, :] = jnp.zeros((8, D), f32)
        th.append(load)
        for r in range(j * TM, (j + 1) * TM, ER):
            def cast(r=r):
                kf[8 + r:8 + r + ER, :] = k_v[r:r + ER, :].astype(f32)
            th.append(cast)
        for b in range(j * BPS, (j + 1) * BPS):
            for r in range(b * B, (b + 1) * B, ER):
                def sconv(r=r):
                    acc = kf[8 + r:8 + r + ER, :] * mod_v[8:9, 0:D]
                    for t in range(1, 4):
                        acc = acc + kf[8 + r - t:8 + r - t + ER, :] * mod_v[8 + t:9 + t, 0:D]
                    kv32[r:r + ER, :] = acc * v_v[r:r + ER, :].astype(f32)
                th.append(sconv)
            def fx(b=b):
                xs[b] = jnp.dot(fwd_v[...], kv32[b * B:(b + 1) * B, :].astype(bf16),
                                preferred_element_type=f32)
            def fh(b=b):
                hraw[b % 2] = jax.lax.dot_general(
                    fwd_v[...], ssmk_v[:, b * B:(b + 1) * B], (((1,), (1,)), ((), ())),
                    preferred_element_type=f32)
            th += [fh, fx]
            for half in range(2):
                def fix(b=b, half=half):
                    re = slice(half * 64, half * 64 + 64)
                    im = slice(B + half * 64, B + half * 64 + 64)
                    cur, prev = hraw.at[b % 2], hraw.at[(b + 1) % 2]
                    if b == 0:
                        hs[b, re, :] = cur[re, :]
                        hs[b, im, :] = cur[im, :]
                    elif half == 0:
                        hs[b, re, :] = cur[re, :] - prev[im, :]
                        hs[b, im, :] = cur[im, :] + prev[re, :]
                    else:
                        hs[b, re, :] = cur[re, :] + prev[im, :]
                        hs[b, im, :] = cur[im, :] - prev[re, :]
                th.append(fix)
        return th

    def stage_b(j):
        th = []
        outs = list(range(j * BPS, (j + 1) * BPS))
        cols = [(c0, min(c0 + MC, D)) for c0 in range(0, D, MC)]
        for r in range(0, B, MR):
            for c0, c1 in cols:
                def mac(r=r, c0=c0, c1=c1):
                    re = slice(r, r + MR)
                    im = slice(B + r, B + r + MR)
                    cs = slice(c0, c1)
                    acc = {}
                    hc = {}
                    for b in range(outs[-1], -1, -1):
                        xr, xi = xs[b, re, cs], xs[b, im, cs]
                        for a in outs:
                            if a < b:
                                continue
                            d = a - b
                            if d not in hc:
                                hc[d] = (hs[d, re, cs], hs[d, im, cs])
                            hr, hi = hc[d]
                            pr = xr * hr - xi * hi
                            pi = xr * hi + xi * hr
                            acc[a] = (pr, pi) if a not in acc else (acc[a][0] + pr, acc[a][1] + pi)
                    for a in outs:
                        zb[a % (2 * BPS), re, cs] = acc[a][0].astype(bf16)
                        zb[a % (2 * BPS), im, cs] = acc[a][1].astype(bf16)
                th.append(mac)
        return th

    def layernorm(x):
        m = jnp.sum(x, axis=-1, keepdims=True) * (1.0 / D)
        xc = x - m
        var = jnp.sum(xc * xc, axis=-1, keepdims=True) * (1.0 / D)
        return xc * jax.lax.rsqrt(var + EPS)

    def mvec(i):
        return mod_v[0:1, i * D:(i + 1) * D]

    def stage_c(j):
        th = [lambda: cp_q[j].wait()]
        p = j % 2
        for a in range(j * BPS, (j + 1) * BPS):
            lo = (a - j * BPS) * B
            def inv(a=a, lo=lo):
                x1[p, lo:lo + B, :] = jnp.dot(inv_v[...], zb[a % (2 * BPS)], preferred_element_type=f32)
            if do_conv:
                th.append(inv)
            for r in range(0, B, ER):
                def ew(a=a, lo=lo, r=r):
                    g = slice(a * B + r, a * B + r + ER)
                    l = slice(lo + r, lo + r + ER)
                    q = q_v[g, :].astype(f32)
                    h = layernorm(q) * (1.0 + mvec(1)) + mvec(0)
                    if do_conv:
                        y = x1[p, l, :] + kv32[g, :] * mod_v[12:13, 0:D]
                    else:
                        y = q
                    x = q + mvec(2) * (h * y)
                    x1[p, l, :] = x
                    hb[p, l, :] = (layernorm(x) * (1.0 + mvec(4)) + mvec(3)).astype(bf16)
                th.append(ew)
        return th

    def stage_d(j):
        th = []
        p = j % 2
        for i in range(NF):
            def gu(i=i):
                if j == 0:
                    cp_w1[i].wait(); cp_w3[i].wait()
                cs = slice(i * FC, (i + 1) * FC)
                h = hb[p]
                g = jnp.dot(h, w1_v[:, cs], preferred_element_type=f32)
                u = jnp.dot(h, w3_v[:, cs], preferred_element_type=f32)
                act[:, cs] = (g * jax.nn.sigmoid(g) * u).astype(bf16)
            th.append(gu)
        for c0 in range(0, D, 128):
            def down(c0=c0):
                if j == 0 and c0 == 0:
                    cp_w2.wait(); modvec(5)
                cs = slice(c0, c0 + 128)
                o = jnp.dot(act[...], w2_v[:, cs], preferred_element_type=f32)
                ob[j * TM:(j + 1) * TM, cs] = (x1[p, :, cs] + mod_v[0:1, 5 * D + c0:5 * D + c0 + 128] * o).astype(bf16)
            th.append(down)
        th.append(lambda: cp_o[j].start())
        return th

    def stage_d_dummy(j):
        def f():
            if j == 0:
                for cp in cp_w1 + cp_w3 + [cp_w2]:
                    cp.wait()
                modvec(5)
            ob[j * TM:(j + 1) * TM, :] = hb[j % 2]
            cp_o[j].start()
        return [f]

    def modvec(i):
        cp_m[i].wait()
        c = c_v[...].astype(f32)
        s = jnp.broadcast_to(c * jax.nn.sigmoid(c), (16, D)).astype(bf16)
        mod_v[0:8, i * D:(i + 1) * D] = jnp.dot(s, wmod_v[:, i * D:(i + 1) * D],
                                                preferred_element_type=f32)[0:8]

    mod_v[8:12, 0:D] = shk_v[...].astype(f32)
    mod_v[12:13, 0:D] = dd_v[...].astype(f32)

    def conv_ab(j):
        if do_conv:
            return stage_a(j), stage_b(j)
        def w():
            cp_k[j].wait(); cp_v[j].wait(); cp_s[j].wait()
        return [w], []

    a, b = conv_ab(0)
    for t in a + b:
        t()
    for i in range(5):
        modvec(i)
    for t in stage_c(0):
        t()
    for j in range(NS):
        d = stage_d(j) if do_ffn else stage_d_dummy(j)
        if j + 1 < NS:
            a, b = conv_ab(j + 1)
            nxt = a + b + stage_c(j + 1)
        else:
            nxt = []
        if CFG['inter']:
            _interleave(d, nxt)
        else:
            for t in nxt + d:
                t()
    for cp in cp_o:
        cp.wait()


@jax.jit
def pallas_adaLN_cond__ssm_conv_h3__glu_gated_swiglu__prompt_kernel(
        A_q, A_k, A_v, A_shift_k, A_ssm_k, A_ssm_D, B_x, B_w1, B_w3, B_w2, c, w_mod):
    del B_x
    TM = CFG['TM']
    fwd, inv = _dft_matrices()
    any_spec = pl.BlockSpec(memory_space=pl.ANY)
    V = pltpu.VMEM
    out = pl.pallas_call(
        _kernel,
        out_shape=jax.ShapeDtypeStruct((S, D), bf16),
        in_specs=[any_spec] * 13,
        out_specs=any_spec,
        scratch_shapes=[
            V((S, D), bf16), V((S, D), bf16), V((S, D), bf16), V((4, D), bf16), V((D, S), bf16),
            V((1, D), bf16), V((D, FF), bf16), V((D, FF), bf16), V((FF, D), bf16), V((1, D), bf16),
            V((D, 6 * D), bf16), V((N2, B), bf16), V((B, N2), bf16),
            V((NB, N2, D), f32), V((NB, N2, D), f32), V((2, N2, D), f32),
            V((8 + S, D), f32), V((S, D), f32), V((2 * TM // B, N2, D), bf16),
            V((2, TM, D), f32), V((2, TM, D), bf16), V((TM, FF), bf16), V((S, D), bf16),
            V((16, 6 * D), f32),
            pltpu.SemaphoreType.DMA((128,)),
        ],
        compiler_params=pltpu.CompilerParams(vmem_limit_bytes=110 * 1024 * 1024),
    )(A_q.reshape(S, D), A_k.reshape(S, D), A_v.reshape(S, D), A_shift_k.T, A_ssm_k,
      A_ssm_D.reshape(1, D), B_w1, B_w3, B_w2, c, w_mod, fwd, inv)
    return out.reshape(1, S, D)
```

```python
import numpy as np
import jax
import jax.numpy as jnp
import jax.experimental.pallas as pl
import jax.experimental.pallas.tpu as pltpu

S, D, FF = 2048, 640, 1536
B = 128
NB = S // B
N2 = 2 * B
ND = D // 128
NF = FF // 128
TM = 256
NS = S // TM
BPS = TM // B
EPS = 1e-5

CFG = dict(MR=16, ER=16, groups=(0, 2, 4, 8), margin=300, lat2=200, mlat=200, t_mac=4200, gap=500, fill=0.2, slack=0, KD=4, dbg=False, tie0=True, tie1=True, scopes=False, only=None)

f32 = jnp.float32
bf16 = jnp.bfloat16
u32 = jnp.uint32


def _dft_matrices(mr):
    f = np.concatenate([np.arange(0, B, 2), np.arange(1, B, 2)])
    ang = 2.0 * np.pi * np.outer(f + 0.5, np.arange(B)) / N2
    fwd = np.concatenate([np.cos(ang), -np.sin(ang)], axis=0)
    order = np.arange(N2).reshape(2, B // mr, mr).transpose(1, 0, 2).reshape(-1)
    inv = fwd[order].T / B
    inv = np.stack([inv[:, :B], inv[:, B:]])
    return fwd.astype(jnp.bfloat16), inv.astype(jnp.bfloat16)


def _ld(ref, *idx):
    return pltpu.bitcast(ref[idx] if idx else ref[...], bf16)


def _token(*xs):
    t = None
    for x in xs:
        x = pltpu.bitcast(x, u32)
        for r in range(0, x.shape[0], 8):
            for c in range(0, x.shape[1], 128):
                w = x[r:r + 8, c:c + 128]
                t = w if t is None else t | w
    return t


def _layernorm(x):
    m = jnp.sum(x, axis=-1, keepdims=True) * (1.0 / D)
    xc = x - m
    var = jnp.sum(xc * xc, axis=-1, keepdims=True) * (1.0 / D)
    return xc * jax.lax.rsqrt(var + EPS)


def _tile(c):
    return slice(c * 128, (c + 1) * 128)


def _kernel(q_hbm, k_hbm, v_hbm, shk_hbm, ssmk_hbm, dd_hbm, w1_hbm, w3_hbm, w2_hbm, c_hbm,
            wmod_hbm, fwd_hbm, inv_hbm, out_hbm,
            q_v, k_v, v_v, shk_v, ssmk_v, dd_v, w1_v, w3_v, w2_v, c_v, wmod_v, fwd_v, inv_v,
            xs, hs, hraw, kf, kv32, zb, x1, hb, act, ob, mod_v, yb, tb, x2, sems, step_sems):
    MR, ER = CFG['MR'], CFG['ER']
    w1_u, w3_u, w2_u, ssmk_u, fwd_u, inv_u, zb_u, hb_u, act_u = [
        r.bitcast(u32) for r in (w1_v, w3_v, w2_v, ssmk_v, fwd_v, inv_v, zb, hb, act)]

    def scope(name, fn):
        if CFG['scopes']:
            with jax.named_scope(name):
                fn()
        else:
            fn()

    nsem = [0]
    def copy(src, dst):
        cp = pltpu.make_async_copy(src, dst, sems.at[nsem[0]])
        nsem[0] += 1
        return cp

    def lanes(i):
        return pl.ds(i * 128 if isinstance(i, int) else pl.multiple_of(i * 128, 128), 128)

    def rows(j):
        return pl.ds(j * TM if isinstance(j, int) else pl.multiple_of(j * TM, TM), TM)

    def step_inputs(j):
        cps = [pltpu.make_async_copy(ssmk_hbm.at[:, lanes(j * BPS + i)], ssmk_v.at[j * BPS + i],
                                     step_sems.at[i * NS + j]) for i in range(BPS)]
        for i, (src, dst) in enumerate(((k_hbm, k_v), (v_hbm, v_v), (q_hbm, q_v))):
            cps.append(pltpu.make_async_copy(src.at[rows(j)], dst.at[j],
                                             step_sems.at[(BPS + i) * NS + j]))
        return cps

    def step_output(j):
        return pltpu.make_async_copy(ob.at[j], out_hbm.at[rows(j)], step_sems.at[(BPS + 3) * NS + j])

    cp_small = [copy(c_hbm, c_v), copy(shk_hbm, shk_v), copy(dd_hbm, dd_v),
                copy(fwd_hbm, fwd_v.at[0]), copy(inv_hbm, inv_v)]
    cp_m = [copy(wmod_hbm.at[:, pl.ds(i * D, D)], wmod_v.at[:, pl.ds(i * D, D)]) for i in range(6)]
    cp_w1 = [copy(w1_hbm.at[:, lanes(i)], w1_v.at[i]) for i in range(NF)]
    cp_w3 = [copy(w3_hbm.at[:, lanes(i)], w3_v.at[i]) for i in range(NF)]
    cp_w2 = [copy(w2_hbm.at[:, lanes(i)], w2_v.at[i]) for i in range(ND)]

    groups = CFG['groups']
    cp_w = [cp_w1[lo:hi] + cp_w3[lo:hi] for lo, hi in zip(groups, groups[1:] + (NF,))]

    def start(cps):
        for cp in cps:
            cp.start()

    def wait(cps):
        for cp in cps:
            cp.wait()

    start(cp_small + step_inputs(0) + cp_m[:1])

    xs[NB] = jnp.zeros((3 * B, D), f32)
    hs[NB] = jnp.zeros((3 * B, D), f32)
    hraw[2 * BPS - 1] = jnp.zeros((N2, D), f32)
    kf[:, TM:, :] = jnp.zeros((ND, 8, 128), f32)

    scope('wait_small', lambda: [cp.wait() for cp in cp_small])

    ones = jnp.uint32(0xFFFFFFFF)
    zero = (fwd_u[0, 0, 0] == ones).astype(jnp.int32)

    def vec(z, i, n, cs=slice(None)):
        m = mod_v[z + i, :, cs]
        return jnp.concatenate([m] * (n // 8), axis=0)

    def modvec(i):
        c = c_v[...].astype(f32)
        s = jnp.broadcast_to(c * jax.nn.sigmoid(c), (16, D)).astype(bf16)
        m = jnp.dot(s, wmod_v[:, i * D:(i + 1) * D], preferred_element_type=f32)[0:8]
        mod_v[i] = 1.0 + m if i in (1, 4) else m

    def transform(j):
        p = j % 2
        z = jnp.minimum(zero, j + 1)
        items = []

        for i in range(BPS):
            for c in range(ND):
                def fh(i=i, c=c):
                    hraw[p * BPS + i, :, _tile(c)] = jax.lax.dot_general(
                        _ld(fwd_u, z), _ld(ssmk_u, j * BPS + i, slice(c * 64, (c + 1) * 64)),
                        (((1,), (1,)), ((), ())), preferred_element_type=f32)
                items.append(('m', [N2], fh))
        def halo():
            kf[:, 0:8, :] = kf[:, TM:, :]
        items.append(('v', 1, halo))
        for i in range(BPS):
            for c in range(ND):
                for r in range(i * B, (i + 1) * B, 4 * ER):
                    def cast(r=r, c=c):
                        kk = k_v[j, r:r + 4 * ER, _tile(c)].astype(f32)
                        kf[c, 8 + r:8 + r + 4 * ER, :] = kk
                        return _token(kk[-8:])
                    items.append(('v', 3 * ER // 4, cast))
        for i in range(BPS):
            for c in range(ND):
                for r in range(i * B, (i + 1) * B, ER):
                    def sconv(r=r, c=c):
                        acc = None
                        for t in range(4):
                            term = kf[z + c, 8 + r - t:8 + r - t + ER, :] * vec(z, 6 + t, ER, _tile(c))
                            acc = term if acc is None else acc + term
                        kv = acc * v_v[j, r:r + ER, _tile(c)].astype(f32)
                        kv32[0, r:r + ER, _tile(c)] = kv
                        return _token(kv)
                    items.append(('v', 10 * ER // 8, sconv))
                def fx(i=i, c=c):
                    x = jnp.dot(_ld(fwd_u, z), kv32[z, i * B:(i + 1) * B, _tile(c)].astype(bf16),
                                preferred_element_type=f32)
                    xs[j * BPS + i, 0:B, _tile(c)] = x[:B] + x[B:]
                    xs[j * BPS + i, B:, _tile(c)] = x
                items.append(('m', [N2], fx))
        items.append(('sync', 0, None))
        for i in range(BPS):
            for r in range(0, B, 8):
                def fix(i=i, r=r):
                    re, im, sm = slice(r, r + 8), slice(B + r, B + r + 8), slice(N2 + r, N2 + r + 8)
                    cur = hraw.at[z + p * BPS + i]
                    prev = hraw.at[z + (p * BPS + i + 2 * BPS - 1) % (2 * BPS)]
                    if r < B // 2:
                        hr, hi = cur[re, :] - prev[im, :], cur[im, :] + prev[re, :]
                    else:
                        hr, hi = cur[re, :] + prev[im, :], cur[im, :] - prev[re, :]
                    hd, hp = hi - hr, hi + hr
                    hs[j * BPS + i, re, :] = hr
                    hs[j * BPS + i, im, :] = hd
                    hs[j * BPS + i, sm, :] = hp
                    return _token(hp)
                items.append(('v', 5 * ND, fix))
        return items

    def finish(j, nt):
        z = jnp.minimum(zero, j + 1)
        items = []
        last = j * BPS + BPS - 1
        xi = [z + jnp.where(d <= last, last - d, NB) for d in range(nt)]
        hi = [z + jnp.where(d <= last, d, NB) for d in range(nt)]
        nterm = sum(nt - (BPS - 1 - i) for i in range(BPS))
        part = {}
        for c in range(ND):
            for r in range(0, B, MR):
                for k in range(3):
                    def mac(r=r, c=c, k=k):
                        rs = slice(k * B + r, k * B + r + MR)
                        acc, h = {}, []
                        for d in range(nt):
                            x = xs[xi[d], rs, _tile(c)]
                            h.append(hs[hi[d], rs, _tile(c)])
                            for i in range(BPS):
                                e = d - (BPS - 1 - i)
                                if e >= 0:
                                    pr = x * h[e]
                                    acc[i] = pr if i not in acc else acc[i] + pr
                        if k < 2:
                            for i in range(BPS):
                                part[i, k] = acc[i]
                            return _token(*acc.values())
                        zs = []
                        for i in range(BPS):
                            zr, zi = part[i, 0] - acc[i], part[i, 0] + part[i, 1]
                            zb[i, c, 2 * r:2 * r + 2 * MR, :] = (
                                jnp.concatenate([zr, zi], axis=0).astype(bf16))
                            zs.append(zr)
                        return _token(*zs)
                    items.append(('v', (2 * nterm + 4) * (MR // 8), mac))
            for i in range(BPS):
                def inv(i=i, c=c):
                    g = jnp.concatenate([_ld(inv_u, z), _ld(inv_u, z + 1)], axis=1)
                    yb[0, i * B:(i + 1) * B, _tile(c)] = jnp.dot(g, _ld(zb_u, z + i, c),
                                                                 preferred_element_type=f32)
                items.append(('m', [B, B], inv))
        pre, post = [], []
        for r in range(0, TM, ER):
            def ew0(r=r):
                q = q_v[j, r:r + ER, :].astype(f32)
                t = (_layernorm(q) * vec(z, 1, ER) + vec(z, 0, ER)) * vec(z, 2, ER)
                tb[0, r:r + ER, :] = t
                x1[0, r:r + ER, :] = q + t * (kv32[z, r:r + ER, :] * vec(z, 10, ER))
                return _token(t[:, D - 128:]) if CFG['tie0'] else None
            def ew1(r=r):
                x = x1[z, r:r + ER, :] + tb[z, r:r + ER, :] * yb[z, r:r + ER, :]
                x2[0, r:r + ER, :] = x
                h = _layernorm(x) * vec(z, 4, ER) + vec(z, 3, ER)
                for c in range(ND):
                    hb[c, r:r + ER, :] = h[:, _tile(c)].astype(bf16)
                return _token(h[:, D - 128:]) if CFG['tie1'] else None
            pre.append(('v', 14 * ER // 8 * ND, ew0))
            post.append(('v', 11 * ER // 8 * ND, ew1))
        return items, pre, post

    def tied(z, tiles, ties):
        cols = []
        for kt, w in enumerate(tiles):
            for g in sorted(ties.get(kt, {})):
                keep = fwd_u[z, 0:8, :] != ones
                parts = [w[:8 * g], jnp.where(keep, w[8 * g:8 * g + 8], ties[kt][g]), w[8 * g + 8:]]
                w = jnp.concatenate([x for x in parts if x.shape[0]], axis=0)
            cols.append(w)
        return pltpu.bitcast(jnp.concatenate(cols, axis=1), bf16)

    def ffn(j, first=False):
        dots = []
        gate, xres = {}, []
        z = jnp.minimum(zero, j + 1)
        for i in range(NF):
            def dot_g(ties, i=i):
                if first and i in groups:
                    n = groups.index(i)
                    wait(cp_w[n])
                    later = cp_w + [step_inputs(2) + cp_w2[:2] + cp_m[5:], cp_w2[2:]]
                    start(later[n + 2])
                    if n == len(groups) - 1:
                        wait(step_inputs(2))
                if i == 0:
                    xres.append(x2[z])
                g = 0.5 * jnp.dot(tied(z, [hb_u[z + c] for c in range(ND)], ties),
                                  _ld(w1_u, z + i), preferred_element_type=f32)
                gate[i] = g * jnp.tanh(g) + g
            def dot_u(ties, i=i):
                u = jnp.dot(tied(z, [hb_u[z + c] for c in range(ND)], ties),
                            _ld(w3_u, z + i), preferred_element_type=f32)
                act[i] = (gate[i] * u).astype(bf16)
            dots += [(ND, dot_g), (ND, dot_u)]
        osum = {}
        for c in range(ND):
            for k0 in range(0, NF, CFG['KD']):
                def down(ties, c=c, k0=k0):
                    if first and c == 0 and k0 == 0:
                        wait(cp_w2 + cp_m[5:])
                        start(step_inputs(3))
                        modvec(5)
                    k1 = k0 + CFG['KD']
                    o = jnp.dot(tied(z, [act_u[i] for i in range(k0, k1)], ties),
                                _ld(w2_u, z + c, slice(k0 * 64, k1 * 64)), preferred_element_type=f32)
                    osum[c] = o if k0 == 0 else osum[c] + o
                    if k1 == NF:
                        res = xres[0][:, _tile(c)] + vec(z, 5, TM, _tile(c)) * osum[c]
                        ob[j, :, _tile(c)] = res.astype(bf16)
                        if c == ND - 1:
                            step_output(j).start()
                dots.append((CFG['KD'], down))
        return dots

    def run_merged(d, nxt):
        total = (sum(nk * TM for nk, _ in d) + sum(sum(c) for k, c, _ in nxt if k == 'm')) / 4
        end = left = 0
        free = [0, 0, 0, 0]
        unit = [0]
        def issue(lengths):
            starts = []
            for n in lengths:
                m = unit[0] % 4
                starts.append(free[m])
                free[m] += n
                unit[0] += 1
            return starts
        pos, now, held, pending = 0, 0.0, [], []
        for n, (nk, dot) in enumerate(d):
            while held and held[0][0] + CFG['mlat'] <= free[unit[0] % 4]:
                kind, c, fn = held.pop(0)[1]
                fn()
                t = issue(c)
                if CFG['dbg']:
                    print('DBG M', fn.__name__, t[0])
            starts = issue([TM] * nk)
            now = max(now, starts[0])
            ties = {}
            while pos < len(nxt):
                kind, c, fn = nxt[pos]
                if kind == 'm':
                    held.append((now, nxt[pos]))
                elif kind == 'until':
                    end, left = total - c, 0
                    for k, cost, _ in nxt[pos + 1:]:
                        if k == 'until':
                            break
                        left += cost if k == 'v' else 0
                elif kind == 'late':
                    if n < c:
                        break
                elif kind == 'sync':
                    if held:
                        break
                    now = max(now, starts[0] + c)
                else:
                    due = now + c * max(end - now, 0) / left
                    if due >= starts[-1] + TM:
                        break
                    tok = fn()
                    now, left = due, left - c
                    if CFG['dbg']:
                        print('DBG', fn.__name__, int(due), starts[0])
                    for n_late, t in enumerate(tok if isinstance(tok, tuple) else (tok,)):
                        if t is not None and n_late * CFG['slack'] < 10000:
                            pending.append((due + n_late * CFG['slack'], t))
                pos += 1
            for due, tok in pending:
                if due < starts[-1] + TM:
                    kt = ([0] + [t for t in range(nk) if starts[t] <= due])[-1]
                    g = int(min(max(due - starts[kt], 0) // 16, TM // 16 - 1))
                    slot = ties.setdefault(kt, {})
                    slot[g] = slot[g] | tok if g in slot else tok
            pending = [x for x in pending if x[0] >= starts[-1] + TM]
            dot(ties)
        run_plain([it for _, it in held] + nxt[pos:])

    def run_plain(items):
        for _, _, fn in items:
            if fn is not None:
                fn()

    def mix(a, b):
        keyed = [((i + 0.5) / len(t), n, i, it) for n, t in enumerate((a, b)) for i, it in enumerate(t)]
        return [e[3] for e in sorted(keyed, key=lambda e: e[:3])]

    taps = shk_v[...].astype(f32)
    for t in range(4):
        mod_v[6 + t] = jnp.broadcast_to(taps[t:t + 1], (8, D))
    mod_v[10] = jnp.broadcast_to(dd_v[...].astype(f32), (8, D))

    def prologue():
        conv, pre, post = finish(0, BPS)
        start(cp_m[1:3])
        run_plain(transform(0))
        wait(cp_m[:1])
        start(cp_m[3:4])
        modvec(0)
        run_plain(conv)
        wait(cp_m[1:3])
        start(cp_m[4:5] + step_inputs(1))
        modvec(1)
        modvec(2)
        run_plain(pre)
        wait(cp_m[3:5])
        start(cp_w[0] + cp_w[1])
        modvec(3)
        modvec(4)
        run_plain(post)
        wait(step_inputs(1))
        run_plain(transform(1))

    def superstep(j, nt, first=False, more=True):
        if more and not first:
            wait(step_inputs(j + 2))
            pl.when(j + 3 < NS)(lambda: start(step_inputs(j + 3)))
        conv, pre, post = finish(j + 1, nt)
        items = [('until', CFG['t_mac'], None)] + mix(pre, conv)
        nxt = transform(j + 2) if more else []
        k = int(len(nxt) * CFG['fill'])
        if first:
            items.append(('late', 2 * groups[-1] + 1, None))
        items += [('until', CFG['t_mac'] - CFG['gap'], None)] + nxt[:k]
        items += [('late', 2 * NF, None), ('sync', CFG['lat2'], None), ('until', CFG['margin'], None)]
        tail = mix(post, nxt[k:]) if more else post
        run_merged(ffn(j, first), items + tail)

    only = CFG['only']
    scope('wait_in0', lambda: [cp.wait() for cp in step_inputs(0)])
    if only is None:
        scope('prologue', prologue)
        scope('step0', lambda: pl.when(zero == 0)(lambda: superstep(0, 2 * BPS, first=True)))
    def body(j, carry):
        superstep(j, (NS - 1) * BPS)
        return carry
    scope('loop', lambda: jax.lax.fori_loop(1, NS - 2, body, 0))
    if only is None:
        scope('step6', lambda: pl.when(zero == 0)(lambda: superstep(NS - 2, NB, more=False)))
        scope('last', lambda: run_merged(ffn(NS - 1), []))
    scope('wait_out', lambda: [step_output(j).wait() for j in range(NS)])


@jax.jit
def pallas_adaLN_cond__ssm_conv_h3__glu_gated_swiglu__prompt_kernel(
        A_q, A_k, A_v, A_shift_k, A_ssm_k, A_ssm_D, B_x, B_w1, B_w3, B_w2, c, w_mod):
    del B_x
    fwd, inv = _dft_matrices(CFG['MR'])
    any_spec = pl.BlockSpec(memory_space=pl.ANY)
    V = pltpu.VMEM
    out = pl.pallas_call(
        _kernel,
        out_shape=jax.ShapeDtypeStruct((S, D), bf16),
        in_specs=[any_spec] * 13,
        out_specs=any_spec,
        scratch_shapes=[
            V((NS, TM, D), bf16), V((NS, TM, D), bf16), V((NS, TM, D), bf16), V((4, D), bf16),
            V((NB, D, B), bf16), V((1, D), bf16), V((NF, D, 128), bf16), V((NF, D, 128), bf16),
            V((ND, FF, 128), bf16), V((1, D), bf16),
            V((D, 6 * D), bf16), V((1, N2, B), bf16), V((2, B, B), bf16),
            V((NB + 1, 3 * B, D), f32), V((NB + 1, 3 * B, D), f32), V((2 * BPS, N2, D), f32),
            V((ND, 8 + TM, 128), f32), V((1, TM, D), f32), V((BPS, ND, N2, 128), bf16),
            V((1, TM, D), f32), V((ND, TM, 128), bf16), V((NF, TM, 128), bf16),
            V((NS, TM, D), bf16), V((11, 8, D), f32),
            V((1, TM, D), f32), V((1, TM, D), f32), V((1, TM, D), f32),
            pltpu.SemaphoreType.DMA((48,)), pltpu.SemaphoreType.DMA(((BPS + 4) * NS,)),
        ],
        compiler_params=pltpu.CompilerParams(vmem_limit_bytes=110 * 1024 * 1024),
    )(A_q.reshape(S, D), A_k.reshape(S, D), A_v.reshape(S, D), A_shift_k.T, A_ssm_k,
      A_ssm_D.reshape(1, D), B_w1, B_w3, B_w2, c, w_mod, fwd, inv)
    return out.reshape(1, S, D)
```

```python
import numpy as np
import jax
import jax.numpy as jnp
import jax.experimental.pallas as pl
import jax.experimental.pallas.tpu as pltpu

S, D, FF = 2048, 640, 1536
B = 128
NB = S // B
N2 = 2 * B
ND = D // 128
NF = FF // 128
TM = 256
NS = S // TM
BPS = TM // B
HALO = 16
EPS = 1e-5

CFG = dict(MR=16, ER=16, groups=(0, 2, 4, 8), margin=300, lat2=200, mlat=200, t_mac=2400, t_post=10400, split=0, reload=False, slack=0, KD=12, dbg=False, ov=0, plan=('a i1', 'i2 m0', 'm1 g0', 'g1 g2 g3', 'd0 d1', '', '', ''), tie0=True, tie1=True, scopes=False, only=None)

f32 = jnp.float32
bf16 = jnp.bfloat16
u32 = jnp.uint32


def _dft_matrices(mr):
    f = np.concatenate([np.arange(0, B, 2), np.arange(1, B, 2)])
    ang = 2.0 * np.pi * np.outer(f + 0.5, np.arange(B)) / N2
    fwd = np.concatenate([np.cos(ang), -np.sin(ang)], axis=0)
    order = np.arange(N2).reshape(2, B // mr, mr).transpose(1, 0, 2).reshape(-1)
    inv = fwd[order].T / B
    inv = np.stack([inv[:, :B], inv[:, B:]])
    return fwd.astype(jnp.bfloat16), inv.astype(jnp.bfloat16)


def _ld(ref, *idx):
    return pltpu.bitcast(ref[idx] if idx else ref[...], bf16)


def _token(*xs):
    t = None
    for x in xs:
        x = pltpu.bitcast(x, u32)
        for r in range(0, x.shape[0], 8):
            for c in range(0, x.shape[1], 128):
                w = x[r:r + 8, c:c + 128]
                t = w if t is None else t | w
    return t


def _layernorm(x):
    m = jnp.sum(x, axis=-1, keepdims=True) * (1.0 / D)
    xc = x - m
    var = jnp.sum(xc * xc, axis=-1, keepdims=True) * (1.0 / D)
    return xc * jax.lax.rsqrt(var + EPS)


def _tile(c):
    return slice(c * 128, (c + 1) * 128)


def _kernel(q_hbm, k_hbm, v_hbm, shk_hbm, ssmk_hbm, dd_hbm, w1_hbm, w3_hbm, w2_hbm, c_hbm,
            wmod_hbm, fwd_hbm, inv_hbm, out_hbm,
            q_v, k_v, v_v, shk_v, ssmk_v, dd_v, w1_v, w3_v, w2_v, c_v, wmod_v, fwd_v, inv_v,
            xs, hs, carry, kv32, zb, hb, act, ob, mod_v, yb, x2, stat, sems, step_sems):
    MR, ER = CFG['MR'], CFG['ER']
    w1_u, w3_u, w2_u, ssmk_u, fwd_u, inv_u, zb_u, hb_u, act_u = [
        r.bitcast(u32) for r in (w1_v, w3_v, w2_v, ssmk_v, fwd_v, inv_v, zb, hb, act)]

    def scope(name, fn):
        if CFG['scopes']:
            with jax.named_scope(name):
                fn()
        else:
            fn()

    nsem = [0]
    def copy(src, dst):
        cp = pltpu.make_async_copy(src, dst, sems.at[nsem[0]])
        nsem[0] += 1
        return cp

    def lanes(i):
        return pl.ds(i * 128 if isinstance(i, int) else pl.multiple_of(i * 128, 128), 128)

    def rows(j, skip=0):
        at = j * TM + skip
        return pl.ds(at if isinstance(j, int) else pl.multiple_of(at, HALO), TM)

    def step_inputs(j):
        cps = [pltpu.make_async_copy(ssmk_hbm.at[:, lanes(j * BPS + i)], ssmk_v.at[j * BPS + i],
                                     step_sems.at[i * NS + j]) for i in range(BPS)]
        for i, (src, dst) in enumerate(((k_hbm, k_v.at[rows(j, HALO)]), (v_hbm, v_v.at[j]),
                                        (q_hbm, q_v.at[j]))):
            cps.append(pltpu.make_async_copy(src.at[rows(j)], dst,
                                             step_sems.at[(BPS + i) * NS + j]))
        return cps

    def step_output(j):
        return pltpu.make_async_copy(ob.at[j], out_hbm.at[rows(j)], step_sems.at[(BPS + 3) * NS + j])

    cp_small = [copy(c_hbm, c_v), copy(shk_hbm, shk_v), copy(dd_hbm, dd_v),
                copy(fwd_hbm, fwd_v.at[0]), copy(inv_hbm, inv_v)]
    cp_m = [copy(wmod_hbm.at[:, pl.ds(i * D, D)], wmod_v.at[:, pl.ds(i * D, D)]) for i in range(6)]
    cp_w1 = [copy(w1_hbm.at[:, lanes(i)], w1_v.at[i]) for i in range(NF)]
    cp_w3 = [copy(w3_hbm.at[:, lanes(i)], w3_v.at[i]) for i in range(NF)]
    cp_w2 = [copy(w2_hbm.at[:, lanes(i)], w2_v.at[i]) for i in range(ND)]

    groups = CFG['groups']
    cp_w = [cp_w1[lo:hi] + cp_w3[lo:hi] for lo, hi in zip(groups, groups[1:] + (NF,))]

    def start(cps):
        for cp in cps:
            cp.start()

    def wait(cps):
        for cp in cps:
            cp.wait()

    stages = dict(a=cp_small + step_inputs(0), m0=cp_m[:3], m1=cp_m[3:5], g0=cp_w[0], g1=cp_w[1], g2=cp_w[2],
                  g3=cp_w[3], i1=step_inputs(1), i2=step_inputs(2), d0=cp_w2[:3] + cp_m[5:], d1=cp_w2[3:])

    def launch(point):
        for name in CFG['plan'][point].split():
            start(stages[name])

    launch(0)

    xs[NB] = jnp.zeros((3 * B, D), f32)
    hs[NB] = jnp.zeros((3 * B, D), f32)
    carry[...] = jnp.zeros((ND, N2, 128), f32)
    k_v[0:HALO, :] = jnp.zeros((HALO, D), bf16)

    scope('wait_small', lambda: [cp.wait() for cp in cp_small])

    ones = jnp.uint32(0xFFFFFFFF)
    zero = (fwd_u[0, 0, 0] == ones).astype(jnp.int32)

    def vec(z, i, n, cs=slice(None)):
        m = mod_v[z + i, :, cs]
        return jnp.concatenate([m] * (n // 8), axis=0)

    def modvec(i):
        c = c_v[...].astype(f32)
        s = jnp.broadcast_to(c * jax.nn.sigmoid(c), (16, D)).astype(bf16)
        m = jnp.dot(s, wmod_v[:, i * D:(i + 1) * D], preferred_element_type=f32)[0:8]
        mod_v[i] = 1.0 + m if i in (1, 4) else m

    def transform(j):
        z = jnp.minimum(zero, j + 1)
        short, spectra = [], []
        for r in range(0, TM, ER):
            for c in range(ND):
                def sconv(r=r, c=c):
                    row = pl.multiple_of(j * TM + r, HALO)
                    kk = k_v[pl.ds(row, HALO + ER), _tile(c)].astype(f32)[HALO - 8:]
                    acc = kk[8:] * vec(z, 6, ER, _tile(c))
                    for t in range(1, 4):
                        acc = acc + pltpu.roll(kk, t, 0)[8:] * vec(z, 6 + t, ER, _tile(c))
                    kv = acc * v_v[j, r:r + ER, _tile(c)].astype(f32)
                    kv32[j, r:r + ER, _tile(c)] = kv
                    return _token(kv)
                short.append(('v', 18 * ER // 8, sconv))
        for i in range(BPS):
            for c in range(ND):
                def fh(i=i, c=c):
                    h = jax.lax.dot_general(
                        _ld(fwd_u, z), _ld(ssmk_u, j * BPS + i, slice(c * 64, (c + 1) * 64)),
                        (((1,), (1,)), ((), ())), preferred_element_type=f32)
                    hs[j * BPS + i, 0:B, _tile(c)] = h[:B]
                    hs[j * BPS + i, B:N2, _tile(c)] = h[B:] - h[:B]
                    hs[j * BPS + i, N2:, _tile(c)] = h[B:] + h[:B]
                def fx(i=i, c=c):
                    x = jnp.dot(_ld(fwd_u, z), kv32[z + j, i * B:(i + 1) * B, _tile(c)].astype(bf16),
                                preferred_element_type=f32)
                    xs[j * BPS + i, 0:B, _tile(c)] = x[:B] + x[B:]
                    xs[j * BPS + i, B:, _tile(c)] = x
                spectra += [('m', [N2], fh), ('m', [N2], fx)]
        return short, spectra

    def convolve(j, nt):
        z = jnp.minimum(zero, j + 1)
        last = j * BPS + BPS - 1
        xi = [z + jnp.where(d <= last, last - d, NB) for d in range(nt)]
        hi = [z + jnp.where(d <= last, d, NB) for d in range(nt)]
        nterm = sum(nt - (BPS - 1 - i) for i in range(BPS))
        items = []
        for c in range(ND):
            for r in range(0, B, MR):
                part = {}
                for k in range(3):
                    def mac(r=r, c=c, k=k, part=part):
                        rs = slice(k * B + r, k * B + r + MR)
                        acc, h = {}, []
                        for d in range(nt):
                            x = xs[xi[d], rs, _tile(c)]
                            h.append(hs[hi[d], rs, _tile(c)])
                            for i in range(BPS):
                                e = d - (BPS - 1 - i)
                                if e >= 0:
                                    pr = x * h[e]
                                    acc[i] = pr if i not in acc else acc[i] + pr
                        if k < 2:
                            part[k] = acc
                            return _token(*acc.values())
                        pr, pi = carry[c, r:r + MR, :], carry[c, B + r:B + r + MR, :]
                        zs = []
                        for i in range(BPS):
                            yr, yi = part[0][i] - acc[i], part[0][i] + part[1][i]
                            zr, zi = (yr - pi, yi + pr) if r < B // 2 else (yr + pi, yi - pr)
                            zb[i, c, 2 * r:2 * r + 2 * MR, :] = (
                                jnp.concatenate([zr, zi], axis=0).astype(bf16))
                            zs.append(zr)
                            pr, pi = yr, yi
                        carry[c, r:r + MR, :] = pr
                        carry[c, B + r:B + r + MR, :] = pi
                        return _token(*zs)
                    items.append(('v', (2 * nterm + 5) * (MR // 8), mac))
            for i in range(BPS):
                def inv(i=i, c=c):
                    g = jnp.concatenate([_ld(inv_u, z), _ld(inv_u, z + 1)], axis=1)
                    yb[0, i * B:(i + 1) * B, _tile(c)] = jnp.dot(g, _ld(zb_u, z + i, c),
                                                                 preferred_element_type=f32)
                items.append(('m', [B, B], inv))
        return items

    def mixing(j):
        z = jnp.minimum(zero, j + 1)
        z2 = jnp.minimum(zero, j + 2)
        pre, post = [], []

        def mean(x):
            return jnp.sum(x, axis=-1, keepdims=True) * (1.0 / D)

        for r in range(0, TM, ER):
            def q_stats(r=r):
                q = q_v[j, r:r + ER, :].astype(f32)
                m = mean(q)
                qc = q - m
                rstd = jnp.broadcast_to(jax.lax.rsqrt(mean(qc * qc) + EPS), (ER, 128))
                stat[0, r:r + ER, :] = jnp.broadcast_to(m, (ER, 128))
                stat[1, r:r + ER, :] = rstd
                return _token(rstd)
            def x_norm(r=r):
                q = q_v[z + j, r:r + ER, :].astype(f32)
                m, rstd = [jnp.concatenate([stat[z + i, r:r + ER, :]] * ND, axis=1) for i in range(2)]
                h = (q - m) * rstd * vec(z, 1, ER) + vec(z, 0, ER)
                y = yb[z, r:r + ER, :] + kv32[z + j, r:r + ER, :] * vec(z, 10, ER)
                x = q + vec(z, 2, ER) * (h * y)
                x2[j, r:r + ER, :] = x
                m = mean(x)
                xc = (x2[z + j, r:r + ER, :] if CFG['reload'] else x) - m
                rstd = jax.lax.rsqrt(mean(xc * xc) + EPS)
                if CFG['reload']:
                    xc = x2[z2 + j, r:r + ER, :] - m
                h = xc * rstd * vec(z, 4, ER) + vec(z, 3, ER)
                for c in range(ND):
                    hb[c, r:r + ER, :] = h[:, _tile(c)].astype(bf16)
                return _token(h[:, D - 128:])
            pre.append(('v', 6 * ER // 8 * ND, q_stats))
            post.append(('v', 19 * ER // 8 * ND, x_norm))
        return pre, post

    def tied(z, tiles, ties):
        cols = []
        for kt, w in enumerate(tiles):
            for g in sorted(ties.get(kt, {})):
                keep = fwd_u[z, 0:8, :] != ones
                parts = [w[:8 * g], jnp.where(keep, w[8 * g:8 * g + 8], ties[kt][g]), w[8 * g + 8:]]
                w = jnp.concatenate([x for x in parts if x.shape[0]], axis=0)
            cols.append(w)
        return pltpu.bitcast(jnp.concatenate(cols, axis=1), bf16)

    def gate_up(j, first=False):
        dots, gate = [], {}
        z = jnp.minimum(zero, j + 1)
        for i in range(NF):
            def dot_g(ties, i=i):
                if first and i in groups:
                    n = groups.index(i)
                    wait(cp_w[n])
                    launch(4 + n)
                g = 0.5 * jnp.dot(tied(z, [hb_u[z + c] for c in range(ND)], ties),
                                  _ld(w1_u, z + i), preferred_element_type=f32)
                gate[i] = g * jnp.tanh(g) + g
            def dot_u(ties, i=i):
                u = jnp.dot(tied(z, [hb_u[z + c] for c in range(ND)], ties),
                            _ld(w3_u, z + i), preferred_element_type=f32)
                act[i] = (gate[i] * u).astype(bf16)
            dots += [(ND, dot_g), (ND, dot_u)]
        return dots

    def down(j):
        dots, osum = [], {}
        z = jnp.minimum(zero, j + 1)
        for c in range(ND):
            for k0 in range(0, NF, CFG['KD']):
                def dot_d(ties, c=c, k0=k0):
                    k1 = k0 + CFG['KD']
                    o = jnp.dot(tied(z, [act_u[z + i] for i in range(k0, k1)], ties),
                                _ld(w2_u, z + c, slice(k0 * 64, k1 * 64)), preferred_element_type=f32)
                    osum[c] = o if k0 == 0 else osum[c] + o
                    if k1 == NF:
                        res = x2[j, :, _tile(c)] + vec(z, 5, TM, _tile(c)) * osum[c]
                        ob[j, :, _tile(c)] = res.astype(bf16)
                dots.append((CFG['KD'], dot_d))
        return dots

    def run_merged(d, nxt):
        total = (sum(nk * TM for nk, _ in d) + sum(sum(c) for k, c, _ in nxt if k == 'm')) / 4
        end = left = 0
        free = [0, 0, 0, 0]
        unit = [0]
        def issue(lengths):
            starts = []
            for n in lengths:
                m = unit[0] % 4
                starts.append(free[m])
                free[m] += n
                unit[0] += 1
            return starts
        pos, now, held, pending = 0, 0.0, [], []
        for n, (nk, dot) in enumerate(d):
            while held and held[0][0] + CFG['mlat'] <= free[unit[0] % 4]:
                kind, c, fn = held.pop(0)[1]
                fn()
                t = issue(c)
                if CFG['dbg']:
                    print('DBG M', fn.__name__, t[0])
            starts = issue([TM] * nk)
            now = max(now, starts[0])
            ties = {}
            while pos < len(nxt):
                kind, c, fn = nxt[pos]
                if kind == 'm':
                    held.append((now, nxt[pos]))
                elif kind == 'until':
                    end, left = total - c, 0
                    for k, cost, _ in nxt[pos + 1:]:
                        if k == 'until':
                            break
                        left += cost if k == 'v' else 0
                elif kind == 'before':
                    pass
                elif kind == 'late':
                    if n < c:
                        break
                elif kind == 'sync':
                    if held:
                        break
                    now = max(now, starts[0] + c)
                else:
                    due = now + c * max(end - now, 0) / left
                    forced = any(k == 'before' and at == n + 1 for k, at, _ in nxt[pos:])
                    if due >= starts[-1] + TM and not forced:
                        break
                    tok = fn()
                    now, left = due, left - c
                    if CFG['dbg']:
                        print('DBG', fn.__name__, int(due), starts[0])
                    for n_late, t in enumerate(tok if isinstance(tok, tuple) else (tok,)):
                        if t is not None and n_late * CFG['slack'] < 10000:
                            pending.append((due + n_late * CFG['slack'], t))
                pos += 1
            for due, tok in pending:
                if due < starts[-1] + TM:
                    kt = ([0] + [t for t in range(nk) if starts[t] <= due])[-1]
                    g = int(min(max(due - starts[kt], 0) // 16, TM // 16 - 1))
                    slot = ties.setdefault(kt, {})
                    slot[g] = slot[g] | tok if g in slot else tok
            pending = [x for x in pending if x[0] >= starts[-1] + TM]
            dot(ties)
        run_plain([it for _, it in held] + nxt[pos:])

    def run_plain(items):
        for _, _, fn in items:
            if fn is not None:
                fn()

    def mix(a, b):
        keyed = [((i + 0.5) / len(t), n, i, it) for n, t in enumerate((a, b)) for i, it in enumerate(t)]
        return [e[3] for e in sorted(keyed, key=lambda e: e[:3])]

    taps = shk_v[...].astype(f32)
    for t in range(4):
        mod_v[6 + t] = jnp.broadcast_to(taps[t:t + 1], (8, D))
    mod_v[10] = jnp.broadcast_to(dd_v[...].astype(f32), (8, D))

    def prologue():
        def early(j, _):
            wait(step_inputs(j))
            pl.when(j == 0)(lambda: launch(1))
            run_plain(sum(transform(j), []))
        jax.lax.fori_loop(0, 3, early, None)
        conv, (pre, post) = convolve(0, BPS), mixing(0)
        launch(2)
        run_plain(conv)
        wait(cp_m[:3])
        for i in range(3):
            modvec(i)
        run_plain(pre)
        wait(cp_m[3:5])
        launch(3)
        modvec(3)
        modvec(4)
        run_plain(post)

    def first_step():
        conv, pre = convolve(1, 2 * BPS), mixing(1)[0]
        items = [('late', 2 * groups[-1] + 1, None), ('until', CFG['margin'], None)] + mix(pre, conv)
        run_merged(gate_up(0, first=True), items)

    def step(j, _):
        ahead = jnp.minimum(j + 2, NS - 1)
        pl.when(j + 2 < NS)(lambda: wait(step_inputs(j + 2)))
        pl.when(j + 3 < NS)(lambda: start(step_inputs(j + 3)))
        post = mixing(j)[1]
        conv, pre = convolve(j + 1, NB), mixing(j + 1)[0]
        dots = down(j - 1)
        k = int(len(conv) * CFG['split'])
        items = [('until', CFG['t_post'], None)] + mix(post, conv[:k]) + [('before', len(dots), None)]
        head, tail = transform(ahead)
        items += [('until', CFG['t_mac'], None)] + mix(pre + head, conv[k:])
        items += [('until', CFG['margin'], None)] + tail
        run_merged(dots + gate_up(j), items)
        step_output(j - 1).start()

    def last_step():
        dots = down(NS - 2)
        items = [('until', 12000, None)] + mixing(NS - 1)[1] + [('before', len(dots), None)]
        run_merged(dots + gate_up(NS - 1), items)
        step_output(NS - 2).start()
        if CFG['ov'] & 4:
            pl.when(zero == 0)(lambda: run_merged(down(NS - 1), []))
        else:
            run_merged(down(NS - 1), [])
        step_output(NS - 1).start()

    only = CFG['only']
    if only is None:
        scope('prologue', prologue)
        scope('step0', (lambda: pl.when(zero == 0)(first_step)) if CFG['ov'] & 2 else first_step)
        def rest():
            wait(cp_w2 + cp_m[5:])
            start(step_inputs(3))
            modvec(5)
        scope('wait_w2', rest)
    scope('loop', lambda: jax.lax.fori_loop(1, NS - 1, step, None))
    if only is None:
        scope('last', (lambda: pl.when(zero == 0)(last_step)) if CFG['ov'] & 1 else last_step)
    scope('wait_out', lambda: [step_output(j).wait() for j in range(NS)])


@jax.jit
def pallas_adaLN_cond__ssm_conv_h3__glu_gated_swiglu__prompt_kernel(
        A_q, A_k, A_v, A_shift_k, A_ssm_k, A_ssm_D, B_x, B_w1, B_w3, B_w2, c, w_mod):
    del B_x
    fwd, inv = _dft_matrices(CFG['MR'])
    any_spec = pl.BlockSpec(memory_space=pl.ANY)
    V = pltpu.VMEM
    out = pl.pallas_call(
        _kernel,
        out_shape=jax.ShapeDtypeStruct((S, D), bf16),
        in_specs=[any_spec] * 13,
        out_specs=any_spec,
        scratch_shapes=[
            V((NS, TM, D), bf16), V((HALO + S, D), bf16), V((NS, TM, D), bf16), V((4, D), bf16),
            V((NB, D, B), bf16), V((1, D), bf16), V((NF, D, 128), bf16), V((NF, D, 128), bf16),
            V((ND, FF, 128), bf16), V((1, D), bf16),
            V((D, 6 * D), bf16), V((1, N2, B), bf16), V((2, B, B), bf16),
            V((NB + 1, 3 * B, D), f32), V((NB + 1, 3 * B, D), f32), V((ND, N2, 128), f32),
            V((NS, TM, D), f32), V((BPS, ND, N2, 128), bf16),
            V((ND, TM, 128), bf16), V((NF, TM, 128), bf16),
            V((NS, TM, D), bf16), V((11, 8, D), f32),
            V((1, TM, D), f32), V((NS, TM, D), f32), V((2, TM, 128), f32),
            pltpu.SemaphoreType.DMA((48,)), pltpu.SemaphoreType.DMA(((BPS + 4) * NS,)),
        ],
        compiler_params=pltpu.CompilerParams(vmem_limit_bytes=110 * 1024 * 1024),
    )(A_q.reshape(S, D), A_k.reshape(S, D), A_v.reshape(S, D), A_shift_k.T, A_ssm_k,
      A_ssm_D.reshape(1, D), B_w1, B_w3, B_w2, c, w_mod, fwd, inv)
    return out.reshape(1, S, D)
```

```python
import numpy as np
import jax
import jax.numpy as jnp
import jax.experimental.pallas as pl
import jax.experimental.pallas.tpu as pltpu

S, D, FF = 2048, 640, 1536
B = 128
NB = S // B
N2 = 2 * B
ND = D // 128
NF = FF // 128
TM = 256
NS = S // TM
BPS = TM // B
HALO = 16
EPS = 1e-5

CFG = dict(MR=16, ER=16, groups=(0, 2, 4, 8), margin=300, lat2=200, mlat=200, t_mac=2400, t_short=1100, early=0, t_post=10600, split=0, reload=False, slack=0, KD=4, GM=256, DM=256, loops=(2,), dbg=False, peel=0, ov=0, plan=('a i1', 'i2 m0', 'm1 g0', 'g1 g2 g3', 'd0 d1', '', '', ''), tie0=True, tie1=True, scopes=False, only=None)

f32 = jnp.float32
bf16 = jnp.bfloat16
u32 = jnp.uint32


def _dft_matrices(mr):
    f = np.concatenate([np.arange(0, B, 2), np.arange(1, B, 2)])
    ang = 2.0 * np.pi * np.outer(f + 0.5, np.arange(B)) / N2
    fwd = np.concatenate([np.cos(ang), -np.sin(ang)], axis=0)
    order = np.arange(N2).reshape(2, B // mr, mr).transpose(1, 0, 2).reshape(-1)
    inv = fwd[order].T / B
    inv = np.stack([inv[:, :B], inv[:, B:]])
    return fwd.astype(jnp.bfloat16), inv.astype(jnp.bfloat16)


def _ld(ref, *idx):
    return pltpu.bitcast(ref[idx] if idx else ref[...], bf16)


def _token(*xs):
    t = None
    for x in xs:
        x = pltpu.bitcast(x, u32)
        for r in range(0, x.shape[0], 8):
            for c in range(0, x.shape[1], 128):
                w = x[r:r + 8, c:c + 128]
                t = w if t is None else t | w
    return t


def _layernorm(x):
    m = jnp.sum(x, axis=-1, keepdims=True) * (1.0 / D)
    xc = x - m
    var = jnp.sum(xc * xc, axis=-1, keepdims=True) * (1.0 / D)
    return xc * jax.lax.rsqrt(var + EPS)


def _tile(c):
    return slice(c * 128, (c + 1) * 128)


def _kernel(q_hbm, k_hbm, v_hbm, shk_hbm, ssmk_hbm, dd_hbm, w1_hbm, w3_hbm, w2_hbm, c_hbm,
            wmod_hbm, fwd_hbm, inv_hbm, out_hbm,
            q_v, k_v, v_v, shk_v, ssmk_v, dd_v, w1_v, w3_v, w2_v, c_v, wmod_v, fwd_v, inv_v,
            xs, hs, carry, kv32, zb, hb, act, ob, mod_v, yb, x2, stat, sems, step_sems):
    MR, ER = CFG['MR'], CFG['ER']
    w1_u, w3_u, w2_u, ssmk_u, fwd_u, inv_u, zb_u, hb_u, act_u = [
        r.bitcast(u32) for r in (w1_v, w3_v, w2_v, ssmk_v, fwd_v, inv_v, zb, hb, act)]

    def scope(name, fn):
        if CFG['scopes']:
            with jax.named_scope(name):
                fn()
        else:
            fn()

    nsem = [0]
    def copy(src, dst):
        cp = pltpu.make_async_copy(src, dst, sems.at[nsem[0]])
        nsem[0] += 1
        return cp

    def lanes(i):
        return pl.ds(i * 128 if isinstance(i, int) else pl.multiple_of(i * 128, 128), 128)

    def rows(j, skip=0):
        at = j * TM + skip
        return pl.ds(at if isinstance(j, int) else pl.multiple_of(at, HALO), TM)

    def step_inputs(j):
        cps = [pltpu.make_async_copy(ssmk_hbm.at[:, lanes(j * BPS + i)], ssmk_v.at[j * BPS + i],
                                     step_sems.at[i * NS + j]) for i in range(BPS)]
        for i, (src, dst) in enumerate(((k_hbm, k_v.at[rows(j, HALO)]), (v_hbm, v_v.at[j]),
                                        (q_hbm, q_v.at[j]))):
            cps.append(pltpu.make_async_copy(src.at[rows(j)], dst,
                                             step_sems.at[(BPS + i) * NS + j]))
        return cps

    def step_output(j):
        return pltpu.make_async_copy(ob.at[j], out_hbm.at[rows(j)], step_sems.at[(BPS + 3) * NS + j])

    cp_small = [copy(c_hbm, c_v), copy(shk_hbm, shk_v), copy(dd_hbm, dd_v),
                copy(fwd_hbm, fwd_v.at[0]), copy(inv_hbm, inv_v)]
    cp_m = [copy(wmod_hbm.at[:, pl.ds(i * D, D)], wmod_v.at[:, pl.ds(i * D, D)]) for i in range(6)]
    cp_w1 = [copy(w1_hbm.at[:, lanes(i)], w1_v.at[i]) for i in range(NF)]
    cp_w3 = [copy(w3_hbm.at[:, lanes(i)], w3_v.at[i]) for i in range(NF)]
    cp_w2 = [copy(w2_hbm.at[:, lanes(i)], w2_v.at[i]) for i in range(ND)]

    cp_last = [copy(ob.at[NS - 1, :, lanes(c)], out_hbm.at[rows(NS - 1), lanes(c)]) for c in range(ND)]

    groups = CFG['groups']
    cp_w = [cp_w1[lo:hi] + cp_w3[lo:hi] for lo, hi in zip(groups, groups[1:] + (NF,))]

    def start(cps):
        for cp in cps:
            cp.start()

    def wait(cps):
        for cp in cps:
            cp.wait()

    stages = dict(a=cp_small + step_inputs(0), m0=cp_m[:3], m1=cp_m[3:5], g0=cp_w[0], g1=cp_w[1], g2=cp_w[2],
                  g3=cp_w[3], i1=step_inputs(1), i2=step_inputs(2), d0=cp_w2[:3] + cp_m[5:], d1=cp_w2[3:])

    def launch(point):
        for name in CFG['plan'][point].split():
            start(stages[name])

    launch(0)

    xs[NB] = jnp.zeros((3 * B, D), f32)
    hs[NB] = jnp.zeros((3 * B, D), f32)
    carry[...] = jnp.zeros((ND, N2, 128), f32)
    k_v[0:HALO, :] = jnp.zeros((HALO, D), bf16)

    scope('wait_small', lambda: [cp.wait() for cp in cp_small])

    ones = jnp.uint32(0xFFFFFFFF)
    zero = (fwd_u[0, 0, 0] == ones).astype(jnp.int32)

    def vec(z, i, n, cs=slice(None)):
        m = mod_v[z + i, :, cs]
        return jnp.concatenate([m] * (n // 8), axis=0)

    def modvec(i):
        c = c_v[...].astype(f32)
        s = jnp.broadcast_to(c * jax.nn.sigmoid(c), (16, D)).astype(bf16)
        m = jnp.dot(s, wmod_v[:, i * D:(i + 1) * D], preferred_element_type=f32)[0:8]
        mod_v[i] = 1.0 + m if i in (1, 4) else m

    def transform(j):
        z = jnp.minimum(zero, j + 1)
        short, spectra = [], []
        for r in range(0, TM, ER):
            for c in range(ND):
                def sconv(r=r, c=c):
                    row = pl.multiple_of(j * TM + r, HALO)
                    kk = k_v[pl.ds(row, HALO + ER), _tile(c)].astype(f32)[HALO - 8:]
                    acc = kk[8:] * vec(z, 6, ER, _tile(c))
                    for t in range(1, 4):
                        acc = acc + pltpu.roll(kk, t, 0)[8:] * vec(z, 6 + t, ER, _tile(c))
                    kv = acc * v_v[j, r:r + ER, _tile(c)].astype(f32)
                    kv32[j, r:r + ER, _tile(c)] = kv
                    return _token(kv)
                short.append(('v', 18 * ER // 8, sconv))
        for i in range(BPS):
            for c in range(ND):
                def fh(i=i, c=c):
                    h = jax.lax.dot_general(
                        _ld(fwd_u, z), _ld(ssmk_u, j * BPS + i, slice(c * 64, (c + 1) * 64)),
                        (((1,), (1,)), ((), ())), preferred_element_type=f32)
                    hs[j * BPS + i, 0:B, _tile(c)] = h[:B]
                    hs[j * BPS + i, B:N2, _tile(c)] = h[B:] - h[:B]
                    hs[j * BPS + i, N2:, _tile(c)] = h[B:] + h[:B]
                def fx(i=i, c=c):
                    x = jnp.dot(_ld(fwd_u, z), kv32[z + j, i * B:(i + 1) * B, _tile(c)].astype(bf16),
                                preferred_element_type=f32)
                    xs[j * BPS + i, 0:B, _tile(c)] = x[:B] + x[B:]
                    xs[j * BPS + i, B:, _tile(c)] = x
                spectra += [('m', [N2], fh), ('m', [N2], fx)]
        return short, spectra

    def convolve(j, nt):
        z = jnp.minimum(zero, j + 1)
        last = j * BPS + BPS - 1
        xi = [z + jnp.where(d <= last, last - d, NB) for d in range(nt)]
        hi = [z + jnp.where(d <= last, d, NB) for d in range(nt)]
        nterm = sum(nt - (BPS - 1 - i) for i in range(BPS))
        items = []
        for c in range(ND):
            for r in range(0, B, MR):
                part = {}
                for k in range(3):
                    def mac(r=r, c=c, k=k, part=part):
                        rs = slice(k * B + r, k * B + r + MR)
                        acc, h = {}, []
                        for d in range(nt):
                            x = xs[xi[d], rs, _tile(c)]
                            h.append(hs[hi[d], rs, _tile(c)])
                            for i in range(BPS):
                                e = d - (BPS - 1 - i)
                                if e >= 0:
                                    pr = x * h[e]
                                    acc[i] = pr if i not in acc else acc[i] + pr
                        if k < 2:
                            part[k] = acc
                            return _token(*acc.values())
                        pr, pi = carry[c, r:r + MR, :], carry[c, B + r:B + r + MR, :]
                        zs = []
                        for i in range(BPS):
                            yr, yi = part[0][i] - acc[i], part[0][i] + part[1][i]
                            zr, zi = (yr - pi, yi + pr) if r < B // 2 else (yr + pi, yi - pr)
                            zb[i, c, 2 * r:2 * r + 2 * MR, :] = (
                                jnp.concatenate([zr, zi], axis=0).astype(bf16))
                            zs.append(zr)
                            pr, pi = yr, yi
                        carry[c, r:r + MR, :] = pr
                        carry[c, B + r:B + r + MR, :] = pi
                        return _token(*zs)
                    items.append(('v', (2 * nterm + 5) * (MR // 8), mac))
            for i in range(BPS):
                def inv(i=i, c=c):
                    g = jnp.concatenate([_ld(inv_u, z), _ld(inv_u, z + 1)], axis=1)
                    yb[0, i * B:(i + 1) * B, _tile(c)] = jnp.dot(g, _ld(zb_u, z + i, c),
                                                                 preferred_element_type=f32)
                items.append(('m', [B, B], inv))
        return items

    def mixing(j):
        z = jnp.minimum(zero, j + 1)
        z2 = jnp.minimum(zero, j + 2)
        pre, post = [], []

        def mean(x):
            return jnp.sum(x, axis=-1, keepdims=True) * (1.0 / D)

        for r in range(0, TM, ER):
            def q_stats(r=r):
                q = q_v[j, r:r + ER, :].astype(f32)
                m = mean(q)
                qc = q - m
                rstd = jnp.broadcast_to(jax.lax.rsqrt(mean(qc * qc) + EPS), (ER, 128))
                stat[0, r:r + ER, :] = jnp.broadcast_to(m, (ER, 128))
                stat[1, r:r + ER, :] = rstd
                return _token(rstd)
            def x_norm(r=r):
                q = q_v[z + j, r:r + ER, :].astype(f32)
                m, rstd = [jnp.concatenate([stat[z + i, r:r + ER, :]] * ND, axis=1) for i in range(2)]
                h = (q - m) * rstd * vec(z, 1, ER) + vec(z, 0, ER)
                y = yb[z, r:r + ER, :] + kv32[z + j, r:r + ER, :] * vec(z, 10, ER)
                x = q + vec(z, 2, ER) * (h * y)
                x2[j, r:r + ER, :] = x
                m = mean(x)
                xc = (x2[z + j, r:r + ER, :] if CFG['reload'] else x) - m
                rstd = jax.lax.rsqrt(mean(xc * xc) + EPS)
                if CFG['reload']:
                    xc = x2[z2 + j, r:r + ER, :] - m
                h = xc * rstd * vec(z, 4, ER) + vec(z, 3, ER)
                for c in range(ND):
                    hb[c, r:r + ER, :] = h[:, _tile(c)].astype(bf16)
                return _token(h[:, D - 128:])
            pre.append(('v', 6 * ER // 8 * ND, q_stats))
            post.append(('v', 19 * ER // 8 * ND, x_norm))
        return pre, post

    def tied(z, tiles, ties):
        cols = []
        for kt, w in enumerate(tiles):
            for g in sorted(ties.get(kt, {})):
                keep = fwd_u[z, 0:8, :] != ones
                parts = [w[:8 * g], jnp.where(keep, w[8 * g:8 * g + 8], ties[kt][g]), w[8 * g + 8:]]
                w = jnp.concatenate([x for x in parts if x.shape[0]], axis=0)
            cols.append(w)
        return pltpu.bitcast(jnp.concatenate(cols, axis=1), bf16)

    def gate_up(j, first=False):
        dots, gate = [], {}
        z = jnp.minimum(zero, j + 1)
        n = CFG['GM']
        for i in range(NF):
            for r in range(0, TM, n):
                zr = jnp.minimum(zero, j + 1 + r)
                def lhs(ties, r=r):
                    return tied(z, [hb_u[z + c, r // 2:(r + n) // 2] for c in range(ND)], ties)
                def dot_g(ties, i=i, r=r, zr=zr, lhs=lhs):
                    if first and r == 0 and i in groups:
                        g = groups.index(i)
                        wait(cp_w[g])
                        launch(4 + g)
                    g = 0.5 * jnp.dot(lhs(ties), _ld(w1_u, zr + i), preferred_element_type=f32)
                    gate[i] = g * jnp.tanh(g) + g
                def dot_u(ties, i=i, r=r, zr=zr, lhs=lhs):
                    u = jnp.dot(lhs(ties), _ld(w3_u, zr + i), preferred_element_type=f32)
                    act[i, r:r + n] = (gate[i] * u).astype(bf16)
                dots += [(ND, n, dot_g), (ND, n, dot_u)]
        return dots

    def down(j, first=False, final=False):
        dots, osum = [], {}
        z = jnp.minimum(zero, j + 1)
        n = CFG['DM']
        for c in range(ND):
            for r in range(0, TM, n):
                zr = jnp.minimum(zero, j + 1 + r)
                for k0 in range(0, NF, CFG['KD']):
                    def dot_d(ties, c=c, r=r, zr=zr, k0=k0):
                        if first and k0 == 0 and r == 0 and c in (0, 3):
                            wait(cp_w2[:3] + cp_m[5:] if c == 0 else cp_w2[3:])
                            if c == 0:
                                start(step_inputs(3))
                                modvec(5)
                        k1 = k0 + CFG['KD']
                        tiles = [act_u[z + i, r // 2:(r + n) // 2] for i in range(k0, k1)]
                        o = jnp.dot(tied(z, tiles, ties), _ld(w2_u, zr + c, slice(k0 * 64, k1 * 64)),
                                    preferred_element_type=f32)
                        osum[c] = o if k0 == 0 else osum[c] + o
                        if k1 == NF:
                            res = x2[j, r:r + n, _tile(c)] + vec(z, 5, n, _tile(c)) * osum[c]
                            ob[j, r:r + n, _tile(c)] = res.astype(bf16)
                            if final and r + n == TM:
                                cp_last[c].start()
                    dots.append((CFG['KD'], n, dot_d))
        return dots

    def run_merged(d, nxt):
        total = (sum(nk * m for nk, m, _ in d) + sum(sum(c) for k, c, _ in nxt if k == 'm')) / 4
        end = left = 0
        free = [0, 0, 0, 0]
        unit = [0]
        def issue(lengths):
            starts = []
            for n in lengths:
                m = unit[0] % 4
                starts.append(free[m])
                free[m] += n
                unit[0] += 1
            return starts
        pos, now, held, pending = 0, 0.0, [], []
        for n, (nk, m_rows, dot) in enumerate(d):
            while held and held[0][0] + CFG['mlat'] <= free[unit[0] % 4]:
                kind, c, fn = held.pop(0)[1]
                fn()
                t = issue(c)
                if CFG['dbg']:
                    print('DBG M', fn.__name__, t[0])
            starts = issue([m_rows] * nk)
            now = max(now, starts[0])
            ties = {}
            while pos < len(nxt):
                kind, c, fn = nxt[pos]
                if kind == 'm':
                    held.append((now, nxt[pos]))
                elif kind == 'until':
                    end, left = total - c, 0
                    for k, cost, _ in nxt[pos + 1:]:
                        if k == 'until':
                            break
                        left += cost if k == 'v' else 0
                elif kind == 'before':
                    pass
                elif kind == 'late':
                    if n < c:
                        break
                elif kind == 'sync':
                    if held:
                        break
                    now = max(now, starts[0] + c)
                else:
                    due = now + c * max(end - now, 0) / max(left, 1)
                    forced = any(k == 'before' and at == n + 1 for k, at, _ in nxt[pos:])
                    if due >= starts[-1] + m_rows and not forced:
                        break
                    tok = fn()
                    now, left = due, left - c
                    if CFG['dbg']:
                        print('DBG', fn.__name__, int(due), starts[0])
                    for n_late, t in enumerate(tok if isinstance(tok, tuple) else (tok,)):
                        if t is not None and n_late * CFG['slack'] < 10000:
                            pending.append((due + n_late * CFG['slack'], t))
                pos += 1
            for due, tok in pending:
                if due < starts[-1] + m_rows:
                    kt = ([0] + [t for t in range(nk) if starts[t] <= due])[-1]
                    g = int(min(max(due - starts[kt], 0) // 16, m_rows // 16 - 1))
                    slot = ties.setdefault(kt, {})
                    slot[g] = slot[g] | tok if g in slot else tok
            pending = [x for x in pending if x[0] >= starts[-1] + m_rows]
            dot(ties)
        run_plain([it for _, it in held] + nxt[pos:])

    def run_plain(items):
        for _, _, fn in items:
            if fn is not None:
                fn()

    def mix(a, b):
        keyed = [((i + 0.5) / max(len(t), 1), n, i, it) for n, t in enumerate((a, b)) for i, it in enumerate(t)]
        return [e[3] for e in sorted(keyed, key=lambda e: e[:3])]

    taps = shk_v[...].astype(f32)
    for t in range(4):
        mod_v[6 + t] = jnp.broadcast_to(taps[t:t + 1], (8, D))
    mod_v[10] = jnp.broadcast_to(dd_v[...].astype(f32).reshape(1, D), (8, D))

    def prologue():
        def early(j, _):
            wait(step_inputs(j))
            pl.when(j == 0)(lambda: launch(1))
            run_plain(sum(transform(j), []))
        jax.lax.fori_loop(0, 3, early, None)
        conv, (pre, post) = convolve(0, BPS), mixing(0)
        launch(2)
        run_plain(conv)
        wait(cp_m[:3])
        for i in range(3):
            modvec(i)
        run_plain(pre)
        wait(cp_m[3:5])
        launch(3)
        modvec(3)
        modvec(4)
        run_plain(post)

    def first_step():
        conv, pre = convolve(1, 2 * BPS), mixing(1)[0]
        items = [('late', 2 * groups[-1] * TM // CFG['GM'] + 1, None), ('until', CFG['margin'], None)] + mix(pre, conv)
        run_merged(gate_up(0, first=True), items)

    def step(j, nt, first=False, more=True):
        ahead = jnp.minimum(j + 2, NS - 1)
        if more and not first:
            pl.when(j + 2 < NS)(lambda: wait(step_inputs(j + 2)))
            pl.when(j + 3 < NS)(lambda: start(step_inputs(j + 3)))
        post = mixing(j)[1]
        conv, pre = convolve(j + 1, nt), mixing(j + 1)[0]
        dots = down(j - 1, first)
        k = int(len(conv) * CFG['split'])
        items = [('until', CFG['t_post'], None)] + mix(post, conv[:k]) + [('before', len(dots), None)]
        head, tail = transform(ahead) if more else ([], [])
        if first:
            items.append(('v', 0, lambda: (wait(step_inputs(j + 2)), start(step_inputs(j + 3)))[0]))
        n = int(len(head) * CFG['early'])
        items += [('until', CFG['t_mac'], None)] + mix(head[:n], conv[k:])
        items += [('until', CFG['t_short'], None)] + mix(head[n:], tail[0::2])
        items += [('until', CFG['margin'], None)] + mix(pre, tail[1::2])
        run_merged(dots + gate_up(j), items)
        step_output(j - 1).start()

    def last_step():
        dots = down(NS - 2)
        items = [('until', 12000, None)] + mixing(NS - 1)[1] + [('before', len(dots), None)]
        run_merged(dots + gate_up(NS - 1), items)
        step_output(NS - 2).start()
        if CFG['ov'] & 4:
            pl.when(zero == 0)(lambda: run_merged(down(NS - 1, final=True), []))
        else:
            run_merged(down(NS - 1, final=True), [])

    only = CFG['only']
    if only is None:
        scope('prologue', prologue)
        scope('step0', (lambda: pl.when(zero == 0)(first_step)) if CFG['ov'] & 2 else first_step)
        if CFG['loops'][0] > 1:
            scope('step1', lambda: step(1, 3 * BPS, first=True))
        else:
            def rest():
                wait(cp_w2 + cp_m[5:])
                start(step_inputs(3))
                modvec(5)
            scope('wait_w2', rest)
    bounds = CFG['loops'] + (NS - 2 if CFG['peel'] else NS - 1,)
    for lo, hi in zip(bounds, bounds[1:]):
        scope(f'loop{lo}', lambda: jax.lax.fori_loop(
            lo, hi, lambda j, _: step(j, (hi + 1) * BPS), None))
    if CFG['peel']:
        f = lambda: step(NS - 2, NB, more=False)
        scope('step6', (lambda: pl.when(zero == 0)(f)) if CFG['peel'] == 2 else f)
    if only is None:
        scope('last', (lambda: pl.when(zero == 0)(last_step)) if CFG['ov'] & 1 else last_step)
    scope('wait_out', lambda: wait([step_output(j) for j in range(NS - 1)] + cp_last))


@jax.jit
def pallas_adaLN_cond__ssm_conv_h3__glu_gated_swiglu__prompt_kernel(
        A_q, A_k, A_v, A_shift_k, A_ssm_k, A_ssm_D, B_x, B_w1, B_w3, B_w2, c, w_mod):
    del B_x
    fwd, inv = _dft_matrices(CFG['MR'])
    any_spec = pl.BlockSpec(memory_space=pl.ANY)
    V = pltpu.VMEM
    out = pl.pallas_call(
        _kernel,
        out_shape=jax.ShapeDtypeStruct((S, D), bf16),
        in_specs=[any_spec] * 13,
        out_specs=any_spec,
        scratch_shapes=[
            V((NS, TM, D), bf16), V((HALO + S, D), bf16), V((NS, TM, D), bf16), V((4, D), bf16),
            V((NB, D, B), bf16), V((D,), bf16), V((NF, D, 128), bf16), V((NF, D, 128), bf16),
            V((ND, FF, 128), bf16), V((1, D), bf16),
            V((D, 6 * D), bf16), V((1, N2, B), bf16), V((2, B, B), bf16),
            V((NB + 1, 3 * B, D), f32), V((NB + 1, 3 * B, D), f32), V((ND, N2, 128), f32),
            V((NS, TM, D), f32), V((BPS, ND, N2, 128), bf16),
            V((ND, TM, 128), bf16), V((NF, TM, 128), bf16),
            V((NS, TM, D), bf16), V((11, 8, D), f32),
            V((1, TM, D), f32), V((NS, TM, D), f32), V((2, TM, 128), f32),
            pltpu.SemaphoreType.DMA((48,)), pltpu.SemaphoreType.DMA(((BPS + 4) * NS,)),
        ],
        compiler_params=pltpu.CompilerParams(vmem_limit_bytes=110 * 1024 * 1024),
    )(A_q.reshape(S, D), A_k.reshape(S, D), A_v.reshape(S, D), A_shift_k.T, A_ssm_k,
      A_ssm_D, B_w1, B_w3, B_w2, c, w_mod, fwd, inv)
    return out.reshape(1, S, D)
```

```python
import numpy as np
import jax
import jax.numpy as jnp
import jax.experimental.pallas as pl
import jax.experimental.pallas.tpu as pltpu

S, D, FF = 2048, 640, 1536
B = 128
NB = S // B
N2 = 2 * B
ND = D // 128
NF = FF // 128
TM = 256
NS = S // TM
BPS = TM // B
HALO = 16
EPS = 1e-5

CFG = dict(MR=16, ER=16, groups=(0, 2, 4, 8), margin=300, lat2=200, mlat=200, t_mac=2400, t_short=1100, early=0, t_post=10600, split=0, reload=False, slack=0, KD=4, GM=256, DM=256, loops=(2,), dbg=False, x1=500, peel=0, ov=0, plan=('a i1', 'i2 m0 m1', 'g0 g1', 'g2 g3', 'd0', 'd1', '', ''), tie0=True, tie1=True, scopes=False, only=None)

f32 = jnp.float32
bf16 = jnp.bfloat16
u32 = jnp.uint32


def _dft_matrices(mr):
    f = np.concatenate([np.arange(0, B, 2), np.arange(1, B, 2)])
    ang = 2.0 * np.pi * np.outer(f + 0.5, np.arange(B)) / N2
    fwd = np.concatenate([np.cos(ang), -np.sin(ang)], axis=0)
    order = np.arange(N2).reshape(2, B // mr, mr).transpose(1, 0, 2).reshape(-1)
    inv = fwd[order].T / B
    inv = np.stack([inv[:, :B], inv[:, B:]])
    return fwd.astype(jnp.bfloat16), inv.astype(jnp.bfloat16)


def _ld(ref, *idx):
    return pltpu.bitcast(ref[idx] if idx else ref[...], bf16)


def _token(*xs):
    t = None
    for x in xs:
        x = pltpu.bitcast(x, u32)
        for r in range(0, x.shape[0], 8):
            for c in range(0, x.shape[1], 128):
                w = x[r:r + 8, c:c + 128]
                t = w if t is None else t | w
    return t


def _layernorm(x):
    m = jnp.sum(x, axis=-1, keepdims=True) * (1.0 / D)
    xc = x - m
    var = jnp.sum(xc * xc, axis=-1, keepdims=True) * (1.0 / D)
    return xc * jax.lax.rsqrt(var + EPS)


def _tile(c):
    return slice(c * 128, (c + 1) * 128)


def _kernel(q_hbm, k_hbm, v_hbm, shk_hbm, ssmk_hbm, dd_hbm, w1_hbm, w3_hbm, w2_hbm, c_hbm,
            wmod_hbm, fwd_hbm, inv_hbm, out_hbm,
            q_v, k_v, v_v, shk_v, ssmk_v, dd_v, w1_v, w3_v, w2_v, c_v, wmod_v, fwd_v, inv_v,
            xs, hs, carry, kv32, zb, hb, act, ob, mod_v, yb, x2, stat, sems, step_sems):
    MR, ER = CFG['MR'], CFG['ER']
    w1_u, w3_u, w2_u, ssmk_u, fwd_u, inv_u, zb_u, hb_u, act_u = [
        r.bitcast(u32) for r in (w1_v, w3_v, w2_v, ssmk_v, fwd_v, inv_v, zb, hb, act)]

    def scope(name, fn):
        if CFG['scopes']:
            with jax.named_scope(name):
                fn()
        else:
            fn()

    nsem = [0]
    def copy(src, dst):
        cp = pltpu.make_async_copy(src, dst, sems.at[nsem[0]])
        nsem[0] += 1
        return cp

    def lanes(i):
        return pl.ds(i * 128 if isinstance(i, int) else pl.multiple_of(i * 128, 128), 128)

    def rows(j, skip=0):
        at = j * TM + skip
        return pl.ds(at if isinstance(j, int) else pl.multiple_of(at, HALO), TM)

    def step_inputs(j):
        cps = [pltpu.make_async_copy(ssmk_hbm.at[:, lanes(j * BPS + i)], ssmk_v.at[j * BPS + i],
                                     step_sems.at[i * NS + j]) for i in range(BPS)]
        for i, (src, dst) in enumerate(((k_hbm, k_v.at[rows(j, HALO)]), (v_hbm, v_v.at[j]),
                                        (q_hbm, q_v.at[j]))):
            cps.append(pltpu.make_async_copy(src.at[rows(j)], dst,
                                             step_sems.at[(BPS + i) * NS + j]))
        return cps

    def step_output(j):
        return pltpu.make_async_copy(ob.at[j], out_hbm.at[rows(j)], step_sems.at[(BPS + 3) * NS + j])

    cp_small = [copy(c_hbm, c_v), copy(shk_hbm, shk_v), copy(dd_hbm, dd_v),
                copy(fwd_hbm, fwd_v.at[0]), copy(inv_hbm, inv_v)]
    cp_m = [copy(wmod_hbm.at[:, pl.ds(i * D, D)], wmod_v.at[:, pl.ds(i * D, D)]) for i in range(6)]
    cp_w1 = [copy(w1_hbm.at[:, lanes(i)], w1_v.at[i]) for i in range(NF)]
    cp_w3 = [copy(w3_hbm.at[:, lanes(i)], w3_v.at[i]) for i in range(NF)]
    cp_w2 = [copy(w2_hbm.at[:, lanes(i)], w2_v.at[i]) for i in range(ND)]

    cp_last = [copy(ob.at[NS - 1, :, lanes(c)], out_hbm.at[rows(NS - 1), lanes(c)]) for c in range(ND)]

    groups = CFG['groups']
    cp_w = [cp_w1[lo:hi] + cp_w3[lo:hi] for lo, hi in zip(groups, groups[1:] + (NF,))]

    def start(cps):
        for cp in cps:
            cp.start()

    def wait(cps):
        for cp in cps:
            cp.wait()

    stages = dict(a=cp_small + step_inputs(0), m0=cp_m[:3], m1=cp_m[3:5], g0=cp_w[0], g1=cp_w[1], g2=cp_w[2],
                  g3=cp_w[3], i1=step_inputs(1), i2=step_inputs(2), d0=cp_w2[:3] + cp_m[5:], d1=cp_w2[3:])

    def launch(point):
        for name in CFG['plan'][point].replace('#', ' ').split():
            start(stages[name])

    launch(0)

    xs[NB] = jnp.zeros((3 * B, D), f32)
    hs[NB] = jnp.zeros((3 * B, D), f32)
    carry[...] = jnp.zeros((ND, N2, 128), f32)
    k_v[0:HALO, :] = jnp.zeros((HALO, D), bf16)

    scope('wait_small', lambda: [cp.wait() for cp in cp_small])

    ones = jnp.uint32(0xFFFFFFFF)
    zero = (fwd_u[0, 0, 0] == ones).astype(jnp.int32)

    def vec(z, i, n, cs=slice(None)):
        m = mod_v[z + i, :, cs]
        return jnp.concatenate([m] * (n // 8), axis=0)

    def modvec(i):
        c = c_v[...].astype(f32)
        s = jnp.broadcast_to(c * jax.nn.sigmoid(c), (16, D)).astype(bf16)
        m = jnp.dot(s, wmod_v[:, i * D:(i + 1) * D], preferred_element_type=f32)[0:8]
        mod_v[i] = 1.0 + m if i in (1, 4) else m

    def transform(j):
        z = jnp.minimum(zero, j + 1)
        short, spectra = [], []
        for r in range(0, TM, ER):
            for c in range(ND):
                def sconv(r=r, c=c):
                    row = pl.multiple_of(j * TM + r, HALO)
                    kk = k_v[pl.ds(row, HALO + ER), _tile(c)].astype(f32)[HALO - 8:]
                    acc = kk[8:] * vec(z, 6, ER, _tile(c))
                    for t in range(1, 4):
                        acc = acc + pltpu.roll(kk, t, 0)[8:] * vec(z, 6 + t, ER, _tile(c))
                    kv = acc * v_v[j, r:r + ER, _tile(c)].astype(f32)
                    kv32[j, r:r + ER, _tile(c)] = kv
                    return _token(kv)
                short.append(('v', 18 * ER // 8, sconv))
        for i in range(BPS):
            for c in range(ND):
                def fh(i=i, c=c):
                    h = jax.lax.dot_general(
                        _ld(fwd_u, z), _ld(ssmk_u, j * BPS + i, slice(c * 64, (c + 1) * 64)),
                        (((1,), (1,)), ((), ())), preferred_element_type=f32)
                    hs[j * BPS + i, 0:B, _tile(c)] = h[:B]
                    hs[j * BPS + i, B:N2, _tile(c)] = h[B:] - h[:B]
                    hs[j * BPS + i, N2:, _tile(c)] = h[B:] + h[:B]
                def fx(i=i, c=c):
                    x = jnp.dot(_ld(fwd_u, z), kv32[z + j, i * B:(i + 1) * B, _tile(c)].astype(bf16),
                                preferred_element_type=f32)
                    xs[j * BPS + i, 0:B, _tile(c)] = x[:B] + x[B:]
                    xs[j * BPS + i, B:, _tile(c)] = x
                spectra += [('m', [N2], fh), ('m', [N2], fx)]
        return short, spectra

    def convolve(j, nt):
        z = jnp.minimum(zero, j + 1)
        last = j * BPS + BPS - 1
        xi = [z + jnp.where(d <= last, last - d, NB) for d in range(nt)]
        hi = [z + jnp.where(d <= last, d, NB) for d in range(nt)]
        nterm = sum(nt - (BPS - 1 - i) for i in range(BPS))
        items = []
        for c in range(ND):
            for r in range(0, B, MR):
                part = {}
                for k in range(3):
                    def mac(r=r, c=c, k=k, part=part):
                        rs = slice(k * B + r, k * B + r + MR)
                        acc, h = {}, []
                        for d in range(nt):
                            x = xs[xi[d], rs, _tile(c)]
                            h.append(hs[hi[d], rs, _tile(c)])
                            for i in range(BPS):
                                e = d - (BPS - 1 - i)
                                if e >= 0:
                                    pr = x * h[e]
                                    acc[i] = pr if i not in acc else acc[i] + pr
                        if k < 2:
                            part[k] = acc
                            return _token(*acc.values())
                        pr, pi = carry[c, r:r + MR, :], carry[c, B + r:B + r + MR, :]
                        zs = []
                        for i in range(BPS):
                            yr, yi = part[0][i] - acc[i], part[0][i] + part[1][i]
                            zr, zi = (yr - pi, yi + pr) if r < B // 2 else (yr + pi, yi - pr)
                            zb[i, c, 2 * r:2 * r + 2 * MR, :] = (
                                jnp.concatenate([zr, zi], axis=0).astype(bf16))
                            zs.append(zr)
                            pr, pi = yr, yi
                        carry[c, r:r + MR, :] = pr
                        carry[c, B + r:B + r + MR, :] = pi
                        return _token(*zs)
                    items.append(('v', (2 * nterm + 5) * (MR // 8), mac))
            for i in range(BPS):
                def inv(i=i, c=c):
                    g = jnp.concatenate([_ld(inv_u, z), _ld(inv_u, z + 1)], axis=1)
                    yb[0, i * B:(i + 1) * B, _tile(c)] = jnp.dot(g, _ld(zb_u, z + i, c),
                                                                 preferred_element_type=f32)
                items.append(('m', [B, B], inv))
        return items

    def mixing(j):
        z = jnp.minimum(zero, j + 1)
        z2 = jnp.minimum(zero, j + 2)
        pre, post = [], []

        def mean(x):
            return jnp.sum(x, axis=-1, keepdims=True) * (1.0 / D)

        for r in range(0, TM, ER):
            def q_stats(r=r):
                q = q_v[j, r:r + ER, :].astype(f32)
                m = mean(q)
                qc = q - m
                rstd = jnp.broadcast_to(jax.lax.rsqrt(mean(qc * qc) + EPS), (ER, 128))
                stat[0, r:r + ER, :] = jnp.broadcast_to(m, (ER, 128))
                stat[1, r:r + ER, :] = rstd
                return _token(rstd)
            def x_norm(r=r):
                q = q_v[z + j, r:r + ER, :].astype(f32)
                m, rstd = [jnp.concatenate([stat[z + i, r:r + ER, :]] * ND, axis=1) for i in range(2)]
                h = (q - m) * rstd * vec(z, 1, ER) + vec(z, 0, ER)
                y = yb[z, r:r + ER, :] + kv32[z + j, r:r + ER, :] * vec(z, 10, ER)
                x = q + vec(z, 2, ER) * (h * y)
                x2[j, r:r + ER, :] = x
                m = mean(x)
                xc = (x2[z + j, r:r + ER, :] if CFG['reload'] else x) - m
                rstd = jax.lax.rsqrt(mean(xc * xc) + EPS)
                if CFG['reload']:
                    xc = x2[z2 + j, r:r + ER, :] - m
                h = xc * rstd * vec(z, 4, ER) + vec(z, 3, ER)
                for c in range(ND):
                    hb[c, r:r + ER, :] = h[:, _tile(c)].astype(bf16)
                return _token(h[:, D - 128:])
            pre.append(('v', 6 * ER // 8 * ND, q_stats))
            post.append(('v', 19 * ER // 8 * ND, x_norm))
        return pre, post

    def tied(z, tiles, ties):
        cols = []
        for kt, w in enumerate(tiles):
            for g in sorted(ties.get(kt, {})):
                keep = fwd_u[z, 0:8, :] != ones
                parts = [w[:8 * g], jnp.where(keep, w[8 * g:8 * g + 8], ties[kt][g]), w[8 * g + 8:]]
                w = jnp.concatenate([x for x in parts if x.shape[0]], axis=0)
            cols.append(w)
        return pltpu.bitcast(jnp.concatenate(cols, axis=1), bf16)

    def gate_up(j, first=False):
        dots, gate = [], {}
        z = jnp.minimum(zero, j + 1)
        n = CFG['GM']
        for i in range(NF):
            for r in range(0, TM, n):
                zr = jnp.minimum(zero, j + 1 + r)
                def lhs(ties, r=r):
                    return tied(z, [hb_u[z + c, r // 2:(r + n) // 2] for c in range(ND)], ties)
                def dot_g(ties, i=i, r=r, zr=zr, lhs=lhs):
                    if first and r == 0 and i in groups:
                        g = groups.index(i)
                        wait(cp_w[g])
                        launch(4 + g)
                    g = 0.5 * jnp.dot(lhs(ties), _ld(w1_u, zr + i), preferred_element_type=f32)
                    gate[i] = g * jnp.tanh(g) + g
                def dot_u(ties, i=i, r=r, zr=zr, lhs=lhs):
                    u = jnp.dot(lhs(ties), _ld(w3_u, zr + i), preferred_element_type=f32)
                    act[i, r:r + n] = (gate[i] * u).astype(bf16)
                dots += [(ND, n, dot_g), (ND, n, dot_u)]
        return dots

    def down(j, first=False, final=False):
        dots, osum = [], {}
        z = jnp.minimum(zero, j + 1)
        n = CFG['DM']
        for c in range(ND):
            for r in range(0, TM, n):
                zr = jnp.minimum(zero, j + 1 + r)
                for k0 in range(0, NF, CFG['KD']):
                    def dot_d(ties, c=c, r=r, zr=zr, k0=k0):
                        if first and k0 == 0 and r == 0 and c in (0, 3):
                            if c == 3:
                                start(sum((step_inputs(t) for t in range(3, NS)), []))
                            wait(cp_w2[:3] + cp_m[5:] if c == 0 else cp_w2[3:])
                            if c == 0:
                                modvec(5)
                        k1 = k0 + CFG['KD']
                        tiles = [act_u[i if final else z + i, r // 2:(r + n) // 2] for i in range(k0, k1)]
                        o = jnp.dot(tied(z, tiles, ties), _ld(w2_u, zr + c, slice(k0 * 64, k1 * 64)),
                                    preferred_element_type=f32)
                        osum[c] = o if k0 == 0 else osum[c] + o
                        if k1 == NF:
                            res = x2[j, r:r + n, _tile(c)] + vec(z, 5, n, _tile(c)) * osum[c]
                            ob[j, r:r + n, _tile(c)] = res.astype(bf16)
                            if final and r + n == TM:
                                cp_last[c].start()
                    dots.append((CFG['KD'], n, dot_d))
        return dots

    def run_merged(d, nxt):
        total = (sum(nk * m for nk, m, _ in d) + sum(sum(c) for k, c, _ in nxt if k == 'm')) / 4
        end = left = 0
        free = [0, 0, 0, 0]
        unit = [0]
        def issue(lengths):
            starts = []
            for n in lengths:
                m = unit[0] % 4
                starts.append(free[m])
                free[m] += n
                unit[0] += 1
            return starts
        pos, now, held, pending = 0, 0.0, [], []
        for n, (nk, m_rows, dot) in enumerate(d):
            while held and held[0][0] + CFG['mlat'] <= free[unit[0] % 4]:
                kind, c, fn = held.pop(0)[1]
                fn()
                t = issue(c)
                if CFG['dbg']:
                    print('DBG M', fn.__name__, t[0])
            starts = issue([m_rows] * nk)
            now = max(now, starts[0])
            ties = {}
            while pos < len(nxt):
                kind, c, fn = nxt[pos]
                if kind == 'm':
                    held.append((now, nxt[pos]))
                elif kind == 'until':
                    end, left = total - c, 0
                    for k, cost, _ in nxt[pos + 1:]:
                        if k == 'until':
                            break
                        left += cost if k == 'v' else 0
                elif kind == 'before':
                    pass
                elif kind == 'late':
                    if n < c:
                        break
                elif kind == 'sync':
                    if held:
                        break
                    now = max(now, starts[0] + c)
                else:
                    due = now + c * max(end - now, 0) / max(left, 1)
                    forced = any(k == 'before' and at == n + 1 for k, at, _ in nxt[pos:])
                    if due >= starts[-1] + m_rows and not forced:
                        break
                    tok = fn()
                    now, left = due, left - c
                    if CFG['dbg']:
                        print('DBG', fn.__name__, int(due), starts[0])
                    for n_late, t in enumerate(tok if isinstance(tok, tuple) else (tok,)):
                        if t is not None and n_late * CFG['slack'] < 10000:
                            pending.append((due + n_late * CFG['slack'], t))
                pos += 1
            for due, tok in pending:
                if due < starts[-1] + m_rows:
                    kt = ([0] + [t for t in range(nk) if starts[t] <= due])[-1]
                    g = int(min(max(due - starts[kt], 0) // 16, m_rows // 16 - 1))
                    slot = ties.setdefault(kt, {})
                    slot[g] = slot[g] | tok if g in slot else tok
            pending = [x for x in pending if x[0] >= starts[-1] + m_rows]
            dot(ties)
        run_plain([it for _, it in held] + nxt[pos:])

    def run_plain(items):
        for _, _, fn in items:
            if fn is not None:
                fn()

    def mix(a, b):
        keyed = [((i + 0.5) / max(len(t), 1), n, i, it) for n, t in enumerate((a, b)) for i, it in enumerate(t)]
        return [e[3] for e in sorted(keyed, key=lambda e: e[:3])]

    taps = shk_v[...].astype(f32)
    for t in range(4):
        mod_v[6 + t] = jnp.broadcast_to(taps[t:t + 1], (8, D))
    mod_v[10] = jnp.broadcast_to(dd_v[...].astype(f32).reshape(1, D), (8, D))

    def prologue():
        def early(j, _):
            wait(step_inputs(j))
            pl.when(j == 0)(lambda: launch(1))
            run_plain(sum(transform(j), []))
        jax.lax.fori_loop(0, 3, early, None)
        conv, (pre, post) = convolve(0, BPS), mixing(0)
        launch(2)
        run_plain(conv)
        wait(cp_m[:3])
        for i in range(3):
            modvec(i)
        run_plain(pre)
        wait(cp_m[3:5])
        launch(3)
        modvec(3)
        modvec(4)
        run_plain(post)

    def first_step():
        conv, pre = convolve(1, 2 * BPS), mixing(1)[0]
        items = [('late', 2 * groups[-1] * TM // CFG['GM'] + 1, None), ('until', CFG['margin'], None)] + mix(pre, conv)
        run_merged(gate_up(0, first=True), items)

    def step(j, nt, first=False, more=True):
        ahead = jnp.minimum(j + 2, NS - 1)
        post = mixing(j)[1]
        conv, pre = convolve(j + 1, nt), mixing(j + 1)[0]
        dots = down(j - 1, first)
        k = int(len(conv) * CFG['split'])
        items = [('until', CFG['t_post'], None)] + mix(post, conv[:k]) + [('before', len(dots), None)]
        head, tail = transform(ahead) if more else ([], [])
        extra = CFG['x1'] if first else 0
        items += [('until', CFG['t_mac'] + 3 * extra, None)] + conv[k:]
        if first:
            items.append(('v', 0, lambda: wait(step_inputs(j + 2))))
        items += [('until', CFG['t_short'] + extra, None)] + mix(head, tail[0::2])
        items += [('until', CFG['margin'], None)] + mix(pre, tail[1::2])
        run_merged(dots + gate_up(j), items)
        step_output(j - 1).start()

    def last_step():
        dots = down(NS - 2)
        items = [('until', 12000, None)] + mixing(NS - 1)[1] + [('before', len(dots), None)]
        mid = [('late', len(dots), None), ('v', 0, lambda: step_output(NS - 2).start())]
        run_merged(dots + gate_up(NS - 1) + down(NS - 1, final=True), items + mid)

    only = CFG['only']
    if only is None:
        scope('prologue', prologue)
        scope('step0', (lambda: pl.when(zero == 0)(first_step)) if CFG['ov'] & 2 else first_step)
        if CFG['loops'][0] > 1:
            scope('step1', lambda: step(1, 3 * BPS, first=True))
        else:
            def rest():
                wait(cp_w2 + cp_m[5:])
                start(step_inputs(3))
                modvec(5)
            scope('wait_w2', rest)
    if only is None:
        wait(sum((step_inputs(t) for t in range(4, NS)), []))
    bounds = CFG['loops'] + (NS - 2 if CFG['peel'] else NS - 1,)
    for lo, hi in zip(bounds, bounds[1:]):
        scope(f'loop{lo}', lambda: jax.lax.fori_loop(
            lo, hi, lambda j, _: step(j, (hi + 1) * BPS), None))
    if CFG['peel']:
        f = lambda: step(NS - 2, NB, more=False)
        scope('step6', (lambda: pl.when(zero == 0)(f)) if CFG['peel'] == 2 else f)
    if only is None:
        scope('last', (lambda: pl.when(zero == 0)(last_step)) if CFG['ov'] & 1 else last_step)
    scope('wait_out', lambda: wait([step_output(j) for j in range(NS - 1)] + cp_last))


@jax.jit
def pallas_adaLN_cond__ssm_conv_h3__glu_gated_swiglu__prompt_kernel(
        A_q, A_k, A_v, A_shift_k, A_ssm_k, A_ssm_D, B_x, B_w1, B_w3, B_w2, c, w_mod):
    del B_x
    fwd, inv = _dft_matrices(CFG['MR'])
    any_spec = pl.BlockSpec(memory_space=pl.ANY)
    V = pltpu.VMEM
    out = pl.pallas_call(
        _kernel,
        out_shape=jax.ShapeDtypeStruct((S, D), bf16),
        in_specs=[any_spec] * 13,
        out_specs=any_spec,
        scratch_shapes=[
            V((NS, TM, D), bf16), V((HALO + S, D), bf16), V((NS, TM, D), bf16), V((4, D), bf16),
            V((NB, D, B), bf16), V((D,), bf16), V((NF, D, 128), bf16), V((NF, D, 128), bf16),
            V((ND, FF, 128), bf16), V((1, D), bf16),
            V((D, 6 * D), bf16), V((1, N2, B), bf16), V((2, B, B), bf16),
            V((NB + 1, 3 * B, D), f32), V((NB + 1, 3 * B, D), f32), V((ND, N2, 128), f32),
            V((NS, TM, D), f32), V((BPS, ND, N2, 128), bf16),
            V((ND, TM, 128), bf16), V((NF, TM, 128), bf16),
            V((NS, TM, D), bf16), V((11, 8, D), f32),
            V((1, TM, D), f32), V((NS, TM, D), f32), V((2, TM, 128), f32),
            pltpu.SemaphoreType.DMA((48,)), pltpu.SemaphoreType.DMA(((BPS + 4) * NS,)),
        ],
        compiler_params=pltpu.CompilerParams(vmem_limit_bytes=110 * 1024 * 1024),
    )(A_q.reshape(S, D), A_k.reshape(S, D), A_v.reshape(S, D), A_shift_k.T, A_ssm_k,
      A_ssm_D, B_w1, B_w3, B_w2, c, w_mod, fwd, inv)
    return out.reshape(1, S, D)
```

```python
import numpy as np
import jax
import jax.numpy as jnp
import jax.experimental.pallas as pl
import jax.experimental.pallas.tpu as pltpu

S, D, FF = 2048, 640, 1536
B = 128
NB = S // B
N2 = 2 * B
ND = D // 128
NF = FF // 128
TM = 256
NS = S // TM
BPS = TM // B
TAPS = 4
HALO = 16
R = 16
KD = 4
EPS = 1e-5
GROUPS = (0, 2, 4, 8)

T_POST, T_CONV, T_SHORT, T_END = 10600, 2400, 1100, 300
OPERAND_LAG = 200

f32 = jnp.float32
bf16 = jnp.bfloat16
u32 = jnp.uint32


def _dft_matrices():
    freq = np.concatenate([np.arange(0, B, 2), np.arange(1, B, 2)])
    angle = 2.0 * np.pi * np.outer(freq + 0.5, np.arange(B)) / N2
    fwd = np.concatenate([np.cos(angle), -np.sin(angle)], axis=0)
    order = np.arange(N2).reshape(2, B // R, R).transpose(1, 0, 2).reshape(-1)
    inv = fwd[order].T / B
    inv = np.stack([inv[:, :B], inv[:, B:]])
    return fwd.astype(bf16), inv.astype(bf16)


def _ld(ref, *idx):
    return pltpu.bitcast(ref[idx], bf16)


def _token(*xs):
    tok = None
    for x in xs:
        x = pltpu.bitcast(x, u32)
        for r in range(0, x.shape[0], 8):
            tok = x[r:r + 8] if tok is None else tok | x[r:r + 8]
    return tok


def _tile(c):
    return slice(c * 128, (c + 1) * 128)


def _mix(a, b):
    keyed = [((i + 0.5) / len(t), n, i) for n, t in enumerate((a, b)) for i in range(len(t))]
    return [(a, b)[n][i] for _, n, i in sorted(keyed)]


def _start(copies):
    for cp in copies:
        cp.start()


def _wait(copies):
    for cp in copies:
        cp.wait()


def _run(items):
    for _, _, fn in items:
        if fn is not None:
            fn()


def _run_under(dots, items):
    total = (sum(nk * TM for nk, _ in dots) + sum(sum(c) for k, c, _ in items if k == 'm')) / 4
    free = [0, 0, 0, 0]
    unit = [0]

    def issue(lengths):
        starts = []
        for n in lengths:
            starts.append(free[unit[0] % 4])
            free[unit[0] % 4] += n
            unit[0] += 1
        return starts

    pos, now, end, left, held = 0, 0.0, 0, 0, []
    for n, (nk, dot) in enumerate(dots):
        while held and held[0][0] + OPERAND_LAG <= free[unit[0] % 4]:
            _, lengths, fn = held.pop(0)[1]
            fn()
            issue(lengths)
        starts = issue([TM] * nk)
        now = max(now, starts[0])
        ties = {}
        while pos < len(items):
            kind, c, fn = items[pos]
            if kind == 'm':
                held.append((now, items[pos]))
            elif kind == 'until':
                end, left = total - c, 0
                for k, cost, _ in items[pos + 1:]:
                    if k == 'until':
                        break
                    left += cost if k == 'v' else 0
            elif kind == 'after':
                if n < c:
                    break
            elif kind == 'v':
                due = now + c * max(end - now, 0) / max(left, 1)
                needed = any(k == 'before' and at == n + 1 for k, at, _ in items[pos:])
                if due >= starts[-1] + TM and not needed:
                    break
                tok = fn()
                now, left = due, left - c
                if tok is not None and due < starts[-1] + TM:
                    kt = max(t for t in range(nk) if t == 0 or starts[t] <= due)
                    g = int(min(max(due - starts[kt], 0) // 16, TM // 16 - 1))
                    slot = ties.setdefault(kt, {})
                    slot[g] = slot[g] | tok if g in slot else tok
            pos += 1
        dot(ties)
    _run([it for _, it in held] + items[pos:])


def _kernel(q_hbm, k_hbm, v_hbm, taps_hbm, filt_hbm, skip_hbm, w1_hbm, w3_hbm, w2_hbm, c_hbm,
            wmod_hbm, fwd_hbm, inv_hbm, out_hbm,
            q_v, k_v, v_v, taps_v, filt_v, skip_v, w1_v, w3_v, w2_v, c_v, wmod_v, fwd_v, inv_v,
            xs, hs, carry, kv, zb, yb, stat, x2, hb, act, ob, vecs, sems, step_sems):
    w1_u, w3_u, w2_u, filt_u, fwd_u, inv_u, zb_u, hb_u, act_u = [
        r.bitcast(u32) for r in (w1_v, w3_v, w2_v, filt_v, fwd_v, inv_v, zb, hb, act)]

    used = []

    def copy(src, dst):
        used.append(None)
        return pltpu.make_async_copy(src, dst, sems.at[len(used) - 1])

    def lanes(i):
        return pl.ds(i * 128 if isinstance(i, int) else pl.multiple_of(i * 128, 128), 128)

    def rows(j, skip=0):
        at = j * TM + skip
        return pl.ds(at if isinstance(j, int) else pl.multiple_of(at, HALO), TM)

    def step_inputs(j):
        pairs = [(filt_hbm.at[:, lanes(j * BPS + i)], filt_v.at[j * BPS + i]) for i in range(BPS)]
        pairs += [(k_hbm.at[rows(j)], k_v.at[rows(j, HALO)]), (v_hbm.at[rows(j)], v_v.at[j]),
                  (q_hbm.at[rows(j)], q_v.at[j])]
        return [pltpu.make_async_copy(src, dst, step_sems.at[i * NS + j])
                for i, (src, dst) in enumerate(pairs)]

    def step_output(j):
        return [pltpu.make_async_copy(ob.at[j], out_hbm.at[rows(j)], step_sems.at[(BPS + 3) * NS + j])]

    cp_small = [copy(c_hbm, c_v), copy(taps_hbm, taps_v), copy(skip_hbm, skip_v),
                copy(fwd_hbm, fwd_v.at[0]), copy(inv_hbm, inv_v)]
    cp_mod = [copy(wmod_hbm.at[:, pl.ds(i * D, D)], wmod_v.at[:, pl.ds(i * D, D)]) for i in range(6)]
    cp_gu = [[copy(src.at[:, lanes(i)], dst.at[i])
              for src, dst in ((w1_hbm, w1_v), (w3_hbm, w3_v)) for i in range(lo, hi)]
             for lo, hi in zip(GROUPS, GROUPS[1:] + (NF,))]
    cp_w2 = [copy(w2_hbm.at[:, lanes(c)], w2_v.at[c]) for c in range(ND)]
    cp_down = [cp_w2[:3] + cp_mod[5:], cp_w2[3:]]
    cp_last = [copy(ob.at[NS - 1, :, lanes(c)], out_hbm.at[rows(NS - 1), lanes(c)]) for c in range(ND)]
    cp_rest = sum((step_inputs(j) for j in range(4, NS)), [])

    _start(cp_small + step_inputs(0) + step_inputs(1))

    xs[NB] = jnp.zeros((3 * B, D), f32)
    hs[NB] = jnp.zeros((3 * B, D), f32)
    carry[...] = jnp.zeros((ND, N2, 128), f32)
    k_v[0:HALO, :] = jnp.zeros((HALO, D), bf16)
    _wait(cp_small)

    ones = jnp.uint32(0xFFFFFFFF)
    opaque = (fwd_u[0, 0, 0] == ones).astype(jnp.int32)

    def zero(j):
        return jnp.minimum(opaque, j + 1)

    SHIFT_A, SCALE_A, GATE_A, SHIFT_B, SCALE_B, GATE_B, TAP0, SKIP = 0, 1, 2, 3, 4, 5, 6, 6 + TAPS
    taps = taps_v[...].astype(f32)
    for t in range(TAPS):
        vecs[TAP0 + t] = jnp.broadcast_to(taps[t:t + 1], (8, D))
    vecs[SKIP] = jnp.broadcast_to(skip_v[...].astype(f32).reshape(1, D), (8, D))

    def modulation(i):
        c = c_v[...].astype(f32)
        s = jnp.broadcast_to(c * jax.nn.sigmoid(c), (16, D)).astype(bf16)
        m = jnp.dot(s, wmod_v[:, i * D:(i + 1) * D], preferred_element_type=f32)[0:8]
        vecs[i] = 1.0 + m if i in (SCALE_A, SCALE_B) else m

    def vec(z, i, n, cols=slice(None)):
        return jnp.concatenate([vecs[z + i, :, cols]] * (n // 8), axis=0)

    def transform(j):
        z = zero(j)
        short, spectra = [], []
        for r in range(0, TM, R):
            for c in range(ND):
                def short_conv(r=r, c=c):
                    row = pl.multiple_of(j * TM + r, HALO)
                    k = k_v[pl.ds(row, HALO + R), _tile(c)].astype(f32)[HALO - 8:]
                    acc = k[8:] * vec(z, TAP0, R, _tile(c))
                    for t in range(1, TAPS):
                        acc = acc + pltpu.roll(k, t, 0)[8:] * vec(z, TAP0 + t, R, _tile(c))
                    gated = acc * v_v[j, r:r + R, _tile(c)].astype(f32)
                    kv[j, r:r + R, _tile(c)] = gated
                    return _token(gated)
                short.append(('v', 18 * R // 8, short_conv))
        for i in range(BPS):
            for c in range(ND):
                def filter_dft(i=i, c=c):
                    h = jax.lax.dot_general(
                        _ld(fwd_u, z), _ld(filt_u, j * BPS + i, slice(c * 64, (c + 1) * 64)),
                        (((1,), (1,)), ((), ())), preferred_element_type=f32)
                    hs[j * BPS + i, 0:B, _tile(c)] = h[:B]
                    hs[j * BPS + i, B:N2, _tile(c)] = h[B:] - h[:B]
                    hs[j * BPS + i, N2:, _tile(c)] = h[B:] + h[:B]

                def input_dft(i=i, c=c):
                    x = jnp.dot(_ld(fwd_u, z), kv[z + j, i * B:(i + 1) * B, _tile(c)].astype(bf16),
                                preferred_element_type=f32)
                    xs[j * BPS + i, 0:B, _tile(c)] = x[:B] + x[B:]
                    xs[j * BPS + i, B:, _tile(c)] = x
                spectra += [('m', [N2], filter_dft), ('m', [N2], input_dft)]
        return short, spectra

    def convolve(j, nt):
        z = zero(j)
        last = j * BPS + BPS - 1
        xi = [z + jnp.where(d <= last, last - d, NB) for d in range(nt)]
        hi = [z + jnp.where(d <= last, d, NB) for d in range(nt)]
        terms = sum(nt - i for i in range(BPS))
        items = []
        for c in range(ND):
            for r in range(0, B, R):
                part = {}
                for k in range(3):
                    def products(r=r, c=c, k=k, part=part):
                        bins = slice(k * B + r, k * B + r + R)
                        acc, h = {}, []
                        for d in range(nt):
                            x = xs[xi[d], bins, _tile(c)]
                            h.append(hs[hi[d], bins, _tile(c)])
                            for i in range(BPS):
                                e = d - (BPS - 1 - i)
                                if e >= 0:
                                    acc[i] = x * h[e] if i not in acc else acc[i] + x * h[e]
                        if k < 2:
                            part[k] = acc
                            return _token(*acc.values())
                        pr, pi = carry[c, r:r + R, :], carry[c, B + r:B + r + R, :]
                        done = []
                        for i in range(BPS):
                            yr, yi = part[0][i] - acc[i], part[0][i] + part[1][i]
                            zr, zi = (yr - pi, yi + pr) if r < B // 2 else (yr + pi, yi - pr)
                            zb[i, c, 2 * r:2 * r + 2 * R, :] = (
                                jnp.concatenate([zr, zi], axis=0).astype(bf16))
                            done.append(zr)
                            pr, pi = yr, yi
                        carry[c, r:r + R, :] = pr
                        carry[c, B + r:B + r + R, :] = pi
                        return _token(*done)
                    items.append(('v', (2 * terms + 5) * (R // 8), products))
            for i in range(BPS):
                def inverse_dft(i=i, c=c):
                    g = jnp.concatenate([_ld(inv_u, z), _ld(inv_u, z + 1)], axis=1)
                    yb[0, i * B:(i + 1) * B, _tile(c)] = jnp.dot(
                        g, _ld(zb_u, z + i, c), preferred_element_type=f32)
                items.append(('m', [B, B], inverse_dft))
        return items

    def mixing(j):
        z = zero(j)
        early, late = [], []

        def mean(x):
            return jnp.sum(x, axis=-1, keepdims=True) * (1.0 / D)

        for r in range(0, TM, R):
            def q_stats(r=r):
                q = q_v[j, r:r + R, :].astype(f32)
                m = mean(q)
                qc = q - m
                rstd = jnp.broadcast_to(jax.lax.rsqrt(mean(qc * qc) + EPS), (R, 128))
                stat[0, r:r + R, :] = jnp.broadcast_to(m, (R, 128))
                stat[1, r:r + R, :] = rstd
                return _token(rstd)

            def residual(r=r):
                q = q_v[z + j, r:r + R, :].astype(f32)
                m, rstd = [jnp.concatenate([stat[z + i, r:r + R, :]] * ND, axis=1) for i in range(2)]
                h = (q - m) * rstd * vec(z, SCALE_A, R) + vec(z, SHIFT_A, R)
                y = yb[z, r:r + R, :] + kv[z + j, r:r + R, :] * vec(z, SKIP, R)
                x = q + vec(z, GATE_A, R) * (h * y)
                x2[j, r:r + R, :] = x
                xc = x - mean(x)
                h = xc * jax.lax.rsqrt(mean(xc * xc) + EPS) * vec(z, SCALE_B, R) + vec(z, SHIFT_B, R)
                for c in range(ND):
                    hb[c, r:r + R, :] = h[:, _tile(c)].astype(bf16)
                return _token(h[:, _tile(ND - 1)])
            early.append(('v', 6 * R // 8 * ND, q_stats))
            late.append(('v', 19 * R // 8 * ND, residual))
        return early, late

    def tied(z, tiles, ties):
        cols = []
        for kt, w in enumerate(tiles):
            for g in sorted(ties.get(kt, {})):
                keep = fwd_u[z, 0:8, :] != ones
                parts = [w[:8 * g], jnp.where(keep, w[8 * g:8 * g + 8], ties[kt][g]), w[8 * g + 8:]]
                w = jnp.concatenate([x for x in parts if x.shape[0]], axis=0)
            cols.append(w)
        return pltpu.bitcast(jnp.concatenate(cols, axis=1), bf16)

    def gate_up(j, first=False):
        dots, gate = [], {}
        z = zero(j)
        for i in range(NF):
            def gate_dot(ties, i=i):
                if first and i in GROUPS:
                    n = GROUPS.index(i)
                    _start(cp_down[n] if n < len(cp_down) else [])
                    _wait(cp_gu[n])
                g = 0.5 * jnp.dot(tied(z, [hb_u[z + c] for c in range(ND)], ties), _ld(w1_u, z + i),
                                  preferred_element_type=f32)
                gate[i] = g * jnp.tanh(g) + g

            def up_dot(ties, i=i):
                u = jnp.dot(tied(z, [hb_u[z + c] for c in range(ND)], ties), _ld(w3_u, z + i),
                            preferred_element_type=f32)
                act[i] = (gate[i] * u).astype(bf16)
            dots += [(ND, gate_dot), (ND, up_dot)]
        return dots

    def down(j, first=False, final=False):
        dots, total = [], {}
        z = zero(j)
        for c in range(ND):
            for k0 in range(0, NF, KD):
                def down_dot(ties, c=c, k0=k0):
                    if first and k0 == 0 and c == 0:
                        _wait(cp_down[0])
                        modulation(GATE_B)
                    if first and k0 == 0 and c == 3:
                        _start(step_inputs(3) + cp_rest)
                        _wait(cp_down[1])
                    tiles = [act_u[i if final else z + i] for i in range(k0, k0 + KD)]
                    o = jnp.dot(tied(z, tiles, ties), _ld(w2_u, z + c, slice(k0 * 64, (k0 + KD) * 64)),
                                preferred_element_type=f32)
                    total[c] = o if k0 == 0 else total[c] + o
                    if k0 + KD == NF:
                        out = x2[j, :, _tile(c)] + vec(z, GATE_B, TM, _tile(c)) * total[c]
                        ob[j, :, _tile(c)] = out.astype(bf16)
                        if final:
                            cp_last[c].start()
                dots.append((KD, down_dot))
        return dots

    def warm_up(j, _):
        pl.when(j == 2)(lambda: _start(cp_gu[0] + cp_gu[1]))
        _wait(step_inputs(j))
        pl.when(j == 0)(lambda: _start(step_inputs(2) + cp_mod[:5]))
        _run(sum(transform(j), []))

    jax.lax.fori_loop(0, 3, warm_up, None)
    early, late = mixing(0)
    _run(convolve(0, BPS))
    _wait(cp_mod[:3])
    for i in range(3):
        modulation(i)
    _run(early)
    _start(cp_gu[2] + cp_gu[3])
    _wait(cp_mod[3:5])
    modulation(SHIFT_B)
    modulation(SCALE_B)
    _run(late)

    _run_under(gate_up(0, first=True),
               [('after', 2 * GROUPS[-1] + 1, None), ('until', T_END, None)]
               + _mix(mixing(1)[0], convolve(1, 2 * BPS)))

    def step(j, nt, first=False):
        dots = down(j - 1, first)
        short, spectra = transform(jnp.minimum(j + 2, NS - 1))
        slack = 500 if first else 0
        items = [('until', T_POST, None)] + mixing(j)[1] + [('before', len(dots), None)]
        items += [('until', T_CONV + 3 * slack, None)] + convolve(j + 1, nt)
        if first:
            items.append(('v', 0, lambda: _wait(step_inputs(j + 2))))
        items += [('until', T_SHORT + slack, None)] + _mix(short, spectra[0::2])
        items += [('until', T_END, None)] + _mix(mixing(j + 1)[0], spectra[1::2])
        _run_under(dots + gate_up(j), items)
        _start(step_output(j - 1))

    step(1, 3 * BPS, first=True)
    _wait(cp_rest)
    jax.lax.fori_loop(2, NS - 1, lambda j, _: step(j, NB), None)

    dots = down(NS - 2)
    _run_under(dots + gate_up(NS - 1) + down(NS - 1, final=True),
               [('until', 12000, None)] + mixing(NS - 1)[1] + [('before', len(dots), None)]
               + [('after', len(dots), None), ('v', 0, lambda: _start(step_output(NS - 2)))])
    _wait(sum((step_output(j) for j in range(NS - 1)), []) + cp_last)


@jax.jit
def pallas_adaLN_cond__ssm_conv_h3__glu_gated_swiglu__prompt_kernel(
        A_q, A_k, A_v, A_shift_k, A_ssm_k, A_ssm_D, B_x, B_w1, B_w3, B_w2, c, w_mod):
    del B_x
    fwd, inv = _dft_matrices()
    hbm = pl.BlockSpec(memory_space=pl.ANY)
    V = pltpu.VMEM
    out = pl.pallas_call(
        _kernel,
        out_shape=jax.ShapeDtypeStruct((S, D), bf16),
        in_specs=[hbm] * 13,
        out_specs=hbm,
        scratch_shapes=[
            V((NS, TM, D), bf16), V((HALO + S, D), bf16), V((NS, TM, D), bf16),
            V((TAPS, D), bf16), V((NB, D, B), bf16), V((D,), bf16),
            V((NF, D, 128), bf16), V((NF, D, 128), bf16), V((ND, FF, 128), bf16),
            V((1, D), bf16), V((D, 6 * D), bf16),
            V((1, N2, B), bf16), V((2, B, B), bf16),
            V((NB + 1, 3 * B, D), f32), V((NB + 1, 3 * B, D), f32),
            V((ND, N2, 128), f32), V((NS, TM, D), f32),
            V((BPS, ND, N2, 128), bf16), V((1, TM, D), f32),
            V((2, TM, 128), f32), V((NS, TM, D), f32),
            V((ND, TM, 128), bf16), V((NF, TM, 128), bf16), V((NS, TM, D), bf16),
            V((7 + TAPS, 8, D), f32),
            pltpu.SemaphoreType.DMA((5 + 6 + 2 * NF + 2 * ND,)),
            pltpu.SemaphoreType.DMA(((BPS + 4) * NS,)),
        ],
        compiler_params=pltpu.CompilerParams(vmem_limit_bytes=110 * 1024 * 1024),
    )(A_q.reshape(S, D), A_k.reshape(S, D), A_v.reshape(S, D), A_shift_k.T, A_ssm_k, A_ssm_D,
      B_w1, B_w3, B_w2, c, w_mod, fwd, inv)
    return out.reshape(1, S, D)
```

```python
import numpy as np
import jax
import jax.numpy as jnp
import jax.experimental.pallas as pl
import jax.experimental.pallas.tpu as pltpu

S, D, FF = 2048, 640, 1536
B = 128
NB = S // B
N2 = 2 * B
ND = D // 128
NF = FF // 128
TM = 256
NS = S // TM
BPS = TM // B
TAPS = 4
HALO = 16
R = 16
KD = 4
EPS = 1e-5
GROUPS = (0, 2, 4, 8)

T_POST, T_CONV, T_SHORT, T_END = 10600, 2400, 1100, 300
OPERAND_LAG = 200

f32 = jnp.float32
bf16 = jnp.bfloat16
u32 = jnp.uint32


def _dft_matrices():
    freq = np.concatenate([np.arange(0, B, 2), np.arange(1, B, 2)])
    angle = 2.0 * np.pi * np.outer(freq + 0.5, np.arange(B)) / N2
    fwd = np.concatenate([np.cos(angle), -np.sin(angle)], axis=0)
    order = np.arange(N2).reshape(2, B // R, R).transpose(1, 0, 2).reshape(-1)
    inv = fwd[order].T / B
    inv = np.stack([inv[:, :B], inv[:, B:]])
    return fwd.astype(bf16), inv.astype(bf16)


def _ld(ref, *idx):
    return pltpu.bitcast(ref[idx], bf16)


def _token(*xs):
    tok = None
    for x in xs:
        x = pltpu.bitcast(x, u32)
        for r in range(0, x.shape[0], 8):
            tok = x[r:r + 8] if tok is None else tok | x[r:r + 8]
    return tok


def _tile(c):
    return slice(c * 128, (c + 1) * 128)


def _mix(a, b):
    keyed = [((i + 0.5) / len(t), n, i) for n, t in enumerate((a, b)) for i in range(len(t))]
    return [(a, b)[n][i] for _, n, i in sorted(keyed)]


def _start(copies):
    for cp in copies:
        cp.start()


def _wait(copies):
    for cp in copies:
        cp.wait()


def _run(items):
    for _, _, fn in items:
        if fn is not None:
            fn()


def _run_under(dots, items):
    total = (sum(nk * TM for nk, _ in dots) + sum(sum(c) for k, c, _ in items if k == 'm')) / 4
    free = [0, 0, 0, 0]
    unit = [0]

    def issue(lengths):
        starts = []
        for n in lengths:
            starts.append(free[unit[0] % 4])
            free[unit[0] % 4] += n
            unit[0] += 1
        return starts

    pos, now, end, left, held = 0, 0.0, 0, 0, []
    for n, (nk, dot) in enumerate(dots):
        while held and held[0][0] + OPERAND_LAG <= free[unit[0] % 4]:
            _, lengths, fn = held.pop(0)[1]
            fn()
            issue(lengths)
        starts = issue([TM] * nk)
        now = max(now, starts[0])
        ties = {}
        while pos < len(items):
            kind, c, fn = items[pos]
            if kind == 'm':
                held.append((now, items[pos]))
            elif kind == 'until':
                end, left = total - c, 0
                for k, cost, _ in items[pos + 1:]:
                    if k == 'until':
                        break
                    left += cost if k == 'v' else 0
            elif kind == 'after':
                if n < c:
                    break
            elif kind == 'v':
                due = now + c * max(end - now, 0) / max(left, 1)
                needed = any(k == 'before' and at == n + 1 for k, at, _ in items[pos:])
                if due >= starts[-1] + TM and not needed:
                    break
                tok = fn()
                now, left = due, left - c
                if tok is not None and due < starts[-1] + TM:
                    kt = max(t for t in range(nk) if t == 0 or starts[t] <= due)
                    g = int(min(max(due - starts[kt], 0) // 16, TM // 16 - 1))
                    slot = ties.setdefault(kt, {})
                    slot[g] = slot[g] | tok if g in slot else tok
            pos += 1
        dot(ties)
    _run([it for _, it in held] + items[pos:])


def _kernel(q_hbm, k_hbm, v_hbm, taps_hbm, filt_hbm, skip_hbm, w1_hbm, w3_hbm, w2_hbm, c_hbm,
            wmod_hbm, fwd_hbm, inv_hbm, out_hbm,
            q_v, k_v, v_v, taps_v, filt_v, skip_v, w1_v, w3_v, w2_v, c_v, wmod_v, fwd_v, inv_v,
            xs, hs, carry, kv, zb, yb, stat, x2, hb, act, ob, vecs, sems, step_sems):
    w1_u, w3_u, w2_u, filt_u, fwd_u, inv_u, zb_u, hb_u, act_u = [
        r.bitcast(u32) for r in (w1_v, w3_v, w2_v, filt_v, fwd_v, inv_v, zb, hb, act)]

    used = []

    def group(pairs):
        used.append(None)
        return [pltpu.make_async_copy(src, dst, sems.at[len(used) - 1]) for src, dst in pairs]

    def lanes(i):
        return pl.ds(i * 128 if isinstance(i, int) else pl.multiple_of(i * 128, 128), 128)

    def rows(j, skip=0):
        at = j * TM + skip
        return pl.ds(at if isinstance(j, int) else pl.multiple_of(at, HALO), TM)

    def input_pairs(j):
        pairs = [(filt_hbm.at[:, lanes(j * BPS + i)], filt_v.at[j * BPS + i]) for i in range(BPS)]
        return pairs + [(k_hbm.at[rows(j)], k_v.at[rows(j, HALO)]), (v_hbm.at[rows(j)], v_v.at[j]),
                        (q_hbm.at[rows(j)], q_v.at[j])]

    def step_inputs(j):
        return [pltpu.make_async_copy(src, dst, step_sems.at[j]) for src, dst in input_pairs(j)]

    mod = [(wmod_hbm.at[:, pl.ds(i * D, D)], wmod_v.at[:, pl.ds(i * D, D)]) for i in range(6)]
    w2 = [(w2_hbm.at[:, lanes(c)], w2_v.at[c]) for c in range(ND)]
    cp_small = group([(c_hbm, c_v), (taps_hbm, taps_v), (skip_hbm, skip_v),
                      (fwd_hbm, fwd_v.at[0]), (inv_hbm, inv_v)])
    cp_mod = [group(mod[:3]), group(mod[3:5])]
    cp_gu = [group([(src.at[:, lanes(i)], dst.at[i])
                    for src, dst in ((w1_hbm, w1_v), (w3_hbm, w3_v)) for i in range(lo, hi)])
             for lo, hi in zip(GROUPS, GROUPS[1:] + (NF,))]
    cp_down = [group(w2[:3] + mod[5:]), group(w2[3:])]
    cp_rest = group(sum((input_pairs(j) for j in range(4, NS)), []))
    cp_out = group([(ob.at[j], out_hbm.at[rows(j)]) for j in range(NS - 1)]
                   + [(ob.at[NS - 1, :, lanes(c)], out_hbm.at[rows(NS - 1), lanes(c)]) for c in range(ND)])

    _start(cp_small + step_inputs(0) + step_inputs(1))

    xs[NB] = jnp.zeros((3 * B, D), f32)
    hs[NB] = jnp.zeros((3 * B, D), f32)
    carry[...] = jnp.zeros((ND, N2, 128), f32)
    k_v[0:HALO, :] = jnp.zeros((HALO, D), bf16)
    _wait(cp_small)

    ones = jnp.uint32(0xFFFFFFFF)
    opaque = (fwd_u[0, 0, 0] == ones).astype(jnp.int32)

    def zero(j):
        return jnp.minimum(opaque, j + 1)

    SHIFT_A, SCALE_A, GATE_A, SHIFT_B, SCALE_B, GATE_B, TAP0, SKIP = 0, 1, 2, 3, 4, 5, 6, 6 + TAPS
    taps = taps_v[...].astype(f32)
    for t in range(TAPS):
        vecs[TAP0 + t] = jnp.broadcast_to(taps[t:t + 1], (8, D))
    vecs[SKIP] = jnp.broadcast_to(skip_v[...].astype(f32).reshape(1, D), (8, D))

    def modulation(i):
        c = c_v[...].astype(f32)
        s = jnp.broadcast_to(c * jax.nn.sigmoid(c), (16, D)).astype(bf16)
        m = jnp.dot(s, wmod_v[:, i * D:(i + 1) * D], preferred_element_type=f32)[0:8]
        vecs[i] = 1.0 + m if i in (SCALE_A, SCALE_B) else m

    def vec(z, i, n, cols=slice(None)):
        return jnp.concatenate([vecs[z + i, :, cols]] * (n // 8), axis=0)

    def transform(j):
        z = zero(j)
        short, spectra = [], []
        for r in range(0, TM, R):
            for c in range(ND):
                def short_conv(r=r, c=c):
                    row = pl.multiple_of(j * TM + r, HALO)
                    k = k_v[pl.ds(row, HALO + R), _tile(c)].astype(f32)[HALO - 8:]
                    acc = k[8:] * vec(z, TAP0, R, _tile(c))
                    for t in range(1, TAPS):
                        acc = acc + pltpu.roll(k, t, 0)[8:] * vec(z, TAP0 + t, R, _tile(c))
                    gated = acc * v_v[j, r:r + R, _tile(c)].astype(f32)
                    kv[j, r:r + R, _tile(c)] = gated
                    return _token(gated)
                short.append(('v', 18 * R // 8, short_conv))
        for i in range(BPS):
            for c in range(ND):
                def filter_dft(i=i, c=c):
                    h = jax.lax.dot_general(
                        _ld(fwd_u, z), _ld(filt_u, j * BPS + i, slice(c * 64, (c + 1) * 64)),
                        (((1,), (1,)), ((), ())), preferred_element_type=f32)
                    hs[j * BPS + i, 0:B, _tile(c)] = h[:B]
                    hs[j * BPS + i, B:N2, _tile(c)] = h[B:] - h[:B]
                    hs[j * BPS + i, N2:, _tile(c)] = h[B:] + h[:B]

                def input_dft(i=i, c=c):
                    x = jnp.dot(_ld(fwd_u, z), kv[z + j, i * B:(i + 1) * B, _tile(c)].astype(bf16),
                                preferred_element_type=f32)
                    xs[j * BPS + i, 0:B, _tile(c)] = x[:B] + x[B:]
                    xs[j * BPS + i, B:, _tile(c)] = x
                spectra += [('m', [N2], filter_dft), ('m', [N2], input_dft)]
        return short, spectra

    def convolve(j, nt):
        z = zero(j)
        last = j * BPS + BPS - 1
        xi = [z + jnp.where(d <= last, last - d, NB) for d in range(nt)]
        hi = [z + jnp.where(d <= last, d, NB) for d in range(nt)]
        terms = sum(nt - i for i in range(BPS))
        items = []
        for c in range(ND):
            for r in range(0, B, R):
                part = {}
                for k in range(3):
                    def products(r=r, c=c, k=k, part=part):
                        bins = slice(k * B + r, k * B + r + R)
                        acc, h = {}, []
                        for d in range(nt):
                            x = xs[xi[d], bins, _tile(c)]
                            h.append(hs[hi[d], bins, _tile(c)])
                            for i in range(BPS):
                                e = d - (BPS - 1 - i)
                                if e >= 0:
                                    acc[i] = x * h[e] if i not in acc else acc[i] + x * h[e]
                        if k < 2:
                            part[k] = acc
                            return _token(*acc.values())
                        pr, pi = carry[c, r:r + R, :], carry[c, B + r:B + r + R, :]
                        done = []
                        for i in range(BPS):
                            yr, yi = part[0][i] - acc[i], part[0][i] + part[1][i]
                            zr, zi = (yr - pi, yi + pr) if r < B // 2 else (yr + pi, yi - pr)
                            zb[i, c, 2 * r:2 * r + 2 * R, :] = (
                                jnp.concatenate([zr, zi], axis=0).astype(bf16))
                            done.append(zr)
                            pr, pi = yr, yi
                        carry[c, r:r + R, :] = pr
                        carry[c, B + r:B + r + R, :] = pi
                        return _token(*done)
                    items.append(('v', (2 * terms + 5) * (R // 8), products))
            for i in range(BPS):
                def inverse_dft(i=i, c=c):
                    g = jnp.concatenate([_ld(inv_u, z), _ld(inv_u, z + 1)], axis=1)
                    yb[0, i * B:(i + 1) * B, _tile(c)] = jnp.dot(
                        g, _ld(zb_u, z + i, c), preferred_element_type=f32)
                items.append(('m', [B, B], inverse_dft))
        return items

    def mixing(j):
        z = zero(j)
        early, late = [], []

        def mean(x):
            return jnp.sum(x, axis=-1, keepdims=True) * (1.0 / D)

        for r in range(0, TM, R):
            def q_stats(r=r):
                q = q_v[j, r:r + R, :].astype(f32)
                m = mean(q)
                qc = q - m
                rstd = jnp.broadcast_to(jax.lax.rsqrt(mean(qc * qc) + EPS), (R, 128))
                stat[0, r:r + R, :] = jnp.broadcast_to(m, (R, 128))
                stat[1, r:r + R, :] = rstd
                return _token(rstd)

            def residual(r=r):
                q = q_v[z + j, r:r + R, :].astype(f32)
                m, rstd = [jnp.concatenate([stat[z + i, r:r + R, :]] * ND, axis=1) for i in range(2)]
                h = (q - m) * rstd * vec(z, SCALE_A, R) + vec(z, SHIFT_A, R)
                y = yb[z, r:r + R, :] + kv[z + j, r:r + R, :] * vec(z, SKIP, R)
                x = q + vec(z, GATE_A, R) * (h * y)
                x2[j, r:r + R, :] = x
                xc = x - mean(x)
                h = xc * jax.lax.rsqrt(mean(xc * xc) + EPS) * vec(z, SCALE_B, R) + vec(z, SHIFT_B, R)
                for c in range(ND):
                    hb[c, r:r + R, :] = h[:, _tile(c)].astype(bf16)
                return _token(h[:, _tile(ND - 1)])
            early.append(('v', 6 * R // 8 * ND, q_stats))
            late.append(('v', 19 * R // 8 * ND, residual))
        return early, late

    def tied(z, tiles, ties):
        cols = []
        for kt, w in enumerate(tiles):
            for g in sorted(ties.get(kt, {})):
                keep = fwd_u[z, 0:8, :] != ones
                parts = [w[:8 * g], jnp.where(keep, w[8 * g:8 * g + 8], ties[kt][g]), w[8 * g + 8:]]
                w = jnp.concatenate([x for x in parts if x.shape[0]], axis=0)
            cols.append(w)
        return pltpu.bitcast(jnp.concatenate(cols, axis=1), bf16)

    def gate_up(j, first=False):
        dots, gate = [], {}
        z = zero(j)
        for i in range(NF):
            def gate_dot(ties, i=i):
                if first and i in GROUPS:
                    n = GROUPS.index(i)
                    _start(cp_down[n] if n < len(cp_down) else [])
                    _wait(cp_gu[n])
                g = 0.5 * jnp.dot(tied(z, [hb_u[z + c] for c in range(ND)], ties), _ld(w1_u, z + i),
                                  preferred_element_type=f32)
                gate[i] = g * jnp.tanh(g) + g

            def up_dot(ties, i=i):
                u = jnp.dot(tied(z, [hb_u[z + c] for c in range(ND)], ties), _ld(w3_u, z + i),
                            preferred_element_type=f32)
                act[i] = (gate[i] * u).astype(bf16)
            dots += [(ND, gate_dot), (ND, up_dot)]
        return dots

    def down(j, first=False, final=False):
        dots, total = [], {}
        z = zero(j)
        for c in range(ND):
            for k0 in range(0, NF, KD):
                def down_dot(ties, c=c, k0=k0):
                    if first and k0 == 0 and c == 0:
                        _wait(cp_down[0])
                        modulation(GATE_B)
                    if first and k0 == 0 and c == 3:
                        _start(step_inputs(3) + cp_rest)
                        _wait(cp_down[1])
                    tiles = [act_u[i if final else z + i] for i in range(k0, k0 + KD)]
                    o = jnp.dot(tied(z, tiles, ties), _ld(w2_u, z + c, slice(k0 * 64, (k0 + KD) * 64)),
                                preferred_element_type=f32)
                    total[c] = o if k0 == 0 else total[c] + o
                    if k0 + KD == NF:
                        out = x2[j, :, _tile(c)] + vec(z, GATE_B, TM, _tile(c)) * total[c]
                        ob[j, :, _tile(c)] = out.astype(bf16)
                        if final:
                            cp_out[NS - 1 + c].start()
                dots.append((KD, down_dot))
        return dots

    def warm_up(j, _):
        pl.when(j == 2)(lambda: _start(cp_gu[0] + cp_gu[1]))
        _wait(step_inputs(j))
        pl.when(j == 0)(lambda: _start(step_inputs(2) + cp_mod[0] + cp_mod[1]))
        _run(sum(transform(j), []))

    jax.lax.fori_loop(0, 3, warm_up, None)
    early, late = mixing(0)
    _run(convolve(0, BPS))
    _wait(cp_mod[0])
    for i in range(3):
        modulation(i)
    _run(early)
    _start(cp_gu[2] + cp_gu[3])
    _wait(cp_mod[1])
    modulation(SHIFT_B)
    modulation(SCALE_B)
    _run(late)

    _run_under(gate_up(0, first=True),
               [('after', 2 * GROUPS[-1] + 1, None), ('until', T_END, None)]
               + _mix(mixing(1)[0], convolve(1, 2 * BPS)))

    def step(j, nt, first=False):
        dots = down(j - 1, first)
        short, spectra = transform(jnp.minimum(j + 2, NS - 1))
        slack = 500 if first else 0
        items = [('until', T_POST, None)] + mixing(j)[1] + [('before', len(dots), None)]
        items += [('until', T_CONV + 3 * slack, None)] + convolve(j + 1, nt)
        if first:
            items.append(('v', 0, lambda: _wait(step_inputs(j + 2))))
        items += [('until', T_SHORT + slack, None)] + _mix(short, spectra[0::2])
        items += [('until', T_END, None)] + _mix(mixing(j + 1)[0], spectra[1::2])
        _run_under(dots + gate_up(j), items)
        pltpu.make_async_copy(ob.at[j - 1], out_hbm.at[rows(j - 1)], sems.at[len(used) - 1]).start()

    step(1, 3 * BPS, first=True)
    _wait(cp_rest)
    jax.lax.fori_loop(2, NS - 1, lambda j, _: step(j, NB), None)

    dots = down(NS - 2)
    _run_under(dots + gate_up(NS - 1) + down(NS - 1, final=True),
               [('until', 12000, None)] + mixing(NS - 1)[1] + [('before', len(dots), None)]
               + [('after', len(dots), None), ('v', 0, lambda: cp_out[NS - 2].start())])
    _wait(cp_out)


@jax.jit
def pallas_adaLN_cond__ssm_conv_h3__glu_gated_swiglu__prompt_kernel(
        A_q, A_k, A_v, A_shift_k, A_ssm_k, A_ssm_D, B_x, B_w1, B_w3, B_w2, c, w_mod):
    del B_x
    fwd, inv = _dft_matrices()
    hbm = pl.BlockSpec(memory_space=pl.ANY)
    V = pltpu.VMEM
    out = pl.pallas_call(
        _kernel,
        out_shape=jax.ShapeDtypeStruct((S, D), bf16),
        in_specs=[hbm] * 13,
        out_specs=hbm,
        scratch_shapes=[
            V((NS, TM, D), bf16), V((HALO + S, D), bf16), V((NS, TM, D), bf16),
            V((TAPS, D), bf16), V((NB, D, B), bf16), V((D,), bf16),
            V((NF, D, 128), bf16), V((NF, D, 128), bf16), V((ND, FF, 128), bf16),
            V((1, D), bf16), V((D, 6 * D), bf16),
            V((1, N2, B), bf16), V((2, B, B), bf16),
            V((NB + 1, 3 * B, D), f32), V((NB + 1, 3 * B, D), f32),
            V((ND, N2, 128), f32), V((NS, TM, D), f32),
            V((BPS, ND, N2, 128), bf16), V((1, TM, D), f32),
            V((2, TM, 128), f32), V((NS, TM, D), f32),
            V((ND, TM, 128), bf16), V((NF, TM, 128), bf16), V((NS, TM, D), bf16),
            V((7 + TAPS, 8, D), f32),
            pltpu.SemaphoreType.DMA((7 + len(GROUPS),)),
            pltpu.SemaphoreType.DMA((4,)),
        ],
        compiler_params=pltpu.CompilerParams(vmem_limit_bytes=110 * 1024 * 1024),
    )(A_q.reshape(S, D), A_k.reshape(S, D), A_v.reshape(S, D), A_shift_k.T, A_ssm_k, A_ssm_D,
      B_w1, B_w3, B_w2, c, w_mod, fwd, inv)
    return out.reshape(1, S, D)
```

```python
import numpy as np
import jax
import jax.numpy as jnp
import jax.experimental.pallas as pl
import jax.experimental.pallas.tpu as pltpu

S, D, FF = 2048, 640, 1536
B = 128
NB = S // B
N2 = 2 * B
ND = D // 128
NF = FF // 128
TM = 256
NS = S // TM
BPS = TM // B
TAPS = 4
HALO = 16
R = 16
KD = 4
EPS = 1e-5
GROUPS = (0, 4, 8)

T_POST, T_CONV, T_SHORT, T_END = 10600, 2450, 1350, 300
OPERAND_LAG = 160

f32 = jnp.float32
bf16 = jnp.bfloat16
u32 = jnp.uint32


def _dft_matrices():
    freq = np.concatenate([np.arange(0, B, 2), np.arange(1, B, 2)])
    angle = 2.0 * np.pi * np.outer(freq + 0.5, np.arange(B)) / N2
    fwd = np.concatenate([np.cos(angle), -np.sin(angle)], axis=0)
    order = np.arange(N2).reshape(2, B // R, R).transpose(1, 0, 2).reshape(-1)
    inv = fwd[order].T / B
    inv = np.stack([inv[:, :B], inv[:, B:]])
    return fwd.astype(bf16), inv.astype(bf16)


def _ld(ref, *idx):
    return pltpu.bitcast(ref[idx], bf16)


def _token(*xs):
    tok = None
    for x in xs:
        x = pltpu.bitcast(x, u32)
        for r in range(0, x.shape[0], 8):
            tok = x[r:r + 8] if tok is None else tok | x[r:r + 8]
    return tok


def _tile(c):
    return slice(c * 128, (c + 1) * 128)


def _mix(a, b):
    keyed = [((i + 0.5) / len(t), n, i) for n, t in enumerate((a, b)) for i in range(len(t))]
    return [(a, b)[n][i] for _, n, i in sorted(keyed)]


def _start(copies):
    for cp in copies:
        cp.start()


def _wait(copies):
    for cp in copies:
        cp.wait()


def _run(items):
    for _, _, fn in items:
        if fn is not None:
            fn()


def _run_under(dots, items):
    total = (sum(nk * TM for nk, _ in dots) + sum(sum(c) for k, c, _ in items if k == 'm')) / 4
    free = [0, 0, 0, 0]
    unit = [0]

    def issue(lengths):
        starts = []
        for n in lengths:
            starts.append(free[unit[0] % 4])
            free[unit[0] % 4] += n
            unit[0] += 1
        return starts

    pos, now, end, left, held = 0, 0.0, 0, 0, []
    for n, (nk, dot) in enumerate(dots):
        while held and held[0][0] + OPERAND_LAG <= free[unit[0] % 4]:
            _, lengths, fn = held.pop(0)[1]
            fn()
            issue(lengths)
        starts = issue([TM] * nk)
        now = max(now, starts[0])
        ties = {}
        while pos < len(items):
            kind, c, fn = items[pos]
            if kind == 'm':
                held.append((now, items[pos]))
            elif kind == 'until':
                end, left = total - c, 0
                for k, cost, _ in items[pos + 1:]:
                    if k == 'until':
                        break
                    left += cost if k == 'v' else 0
            elif kind == 'after':
                if n < c:
                    break
            elif kind == 'v':
                due = now + c * max(end - now, 0) / max(left, 1)
                needed = any(k == 'before' and at == n + 1 for k, at, _ in items[pos:])
                if due >= starts[-1] + TM and not needed:
                    break
                tok = fn()
                now, left = due, left - c
                if tok is not None and due < starts[-1] + TM:
                    kt = max(t for t in range(nk) if t == 0 or starts[t] <= due)
                    g = int(min(max(due - starts[kt], 0) // 16, TM // 16 - 1))
                    slot = ties.setdefault(kt, {})
                    slot[g] = slot[g] | tok if g in slot else tok
            pos += 1
        dot(ties)
    _run([it for _, it in held] + items[pos:])


def _kernel(q_hbm, k_hbm, v_hbm, taps_hbm, filt_hbm, skip_hbm, w1_hbm, w3_hbm, w2_hbm, c_hbm,
            wmod_hbm, fwd_hbm, inv_hbm, out_hbm,
            q_v, k_v, v_v, taps_v, filt_v, skip_v, w1_v, w3_v, w2_v, c_v, wmod_v, fwd_v, inv_v,
            xs, hs, carry, kv, zb, yb, stat, x2, hb, act, ob, vecs, sems, step_sems):
    w1_u, w3_u, w2_u, filt_u, fwd_u, inv_u, zb_u, hb_u, act_u = [
        r.bitcast(u32) for r in (w1_v, w3_v, w2_v, filt_v, fwd_v, inv_v, zb, hb, act)]

    used = []

    def group(pairs):
        used.append(None)
        return [pltpu.make_async_copy(src, dst, sems.at[len(used) - 1]) for src, dst in pairs]

    def lanes(i):
        return pl.ds(i * 128 if isinstance(i, int) else pl.multiple_of(i * 128, 128), 128)

    def rows(j, skip=0):
        at = j * TM + skip
        return pl.ds(at if isinstance(j, int) else pl.multiple_of(at, HALO), TM)

    def input_pairs(j):
        pairs = [(filt_hbm.at[:, lanes(j * BPS + i)], filt_v.at[j * BPS + i]) for i in range(BPS)]
        return pairs + [(k_hbm.at[rows(j)], k_v.at[rows(j, HALO)]), (v_hbm.at[rows(j)], v_v.at[j]),
                        (q_hbm.at[rows(j)], q_v.at[j])]

    def step_inputs(j):
        return [pltpu.make_async_copy(src, dst, step_sems.at[j]) for src, dst in input_pairs(j)]

    mod = [(wmod_hbm.at[:, pl.ds(i * D, D)], wmod_v.at[:, pl.ds(i * D, D)]) for i in range(6)]
    w2 = [(w2_hbm.at[:, lanes(c)], w2_v.at[c]) for c in range(ND)]
    cp_small = group([(c_hbm, c_v), (taps_hbm, taps_v), (skip_hbm, skip_v),
                      (fwd_hbm, fwd_v.at[0]), (inv_hbm, inv_v)])
    cp_mod = [group([(wmod_hbm.at[:, pl.ds(lo * D, n * D)], wmod_v.at[:, pl.ds(lo * D, n * D)])])
              for lo, n in ((0, 3), (3, 2))]
    cp_gu = [group([(src.at[:, lanes(i)], dst.at[i])
                    for src, dst in ((w1_hbm, w1_v), (w3_hbm, w3_v)) for i in range(lo, hi)])
             for lo, hi in zip(GROUPS, GROUPS[1:] + (NF,))]
    cp_down = [group(w2[:3] + mod[5:]), group(w2[3:])]
    cp_rest = group(sum((input_pairs(j) for j in range(4, NS)), []))
    cp_out = group([(ob.at[j], out_hbm.at[rows(j)]) for j in range(NS - 1)]
                   + [(ob.at[NS - 1, :, lanes(c)], out_hbm.at[rows(NS - 1), lanes(c)]) for c in range(ND)])

    _start(cp_small + step_inputs(0))

    xs[NB] = jnp.zeros((3 * B, D), f32)
    hs[NB] = jnp.zeros((3 * B, D), f32)
    carry[...] = jnp.zeros((ND, N2, 128), f32)
    k_v[0:HALO, :] = jnp.zeros((HALO, D), bf16)
    _wait(cp_small)

    ones = jnp.uint32(0xFFFFFFFF)
    opaque = (fwd_u[0, 0, 0] == ones).astype(jnp.int32)

    def zero(j):
        return jnp.minimum(opaque, j + 1)

    SHIFT_A, SCALE_A, GATE_A, SHIFT_B, SCALE_B, GATE_B, TAP0, SKIP = 0, 1, 2, 3, 4, 5, 6, 6 + TAPS
    taps = taps_v[...].astype(f32)
    for t in range(TAPS):
        vecs[TAP0 + t] = jnp.broadcast_to(taps[t:t + 1], (8, D))
    vecs[SKIP] = jnp.broadcast_to(skip_v[...].astype(f32).reshape(1, D), (8, D))

    def modulation(i):
        c = c_v[...].astype(f32)
        s = jnp.broadcast_to(c * jax.nn.sigmoid(c), (16, D)).astype(bf16)
        m = jnp.dot(s, wmod_v[:, i * D:(i + 1) * D], preferred_element_type=f32)[0:8]
        vecs[i] = 1.0 + m if i in (SCALE_A, SCALE_B) else m

    def vec(z, i, n, cols=slice(None)):
        return jnp.concatenate([vecs[z + i, :, cols]] * (n // 8), axis=0)

    def transform(j):
        z = zero(j)
        short, spectra = [], []
        for r in range(0, TM, R):
            for c in range(ND):
                def short_conv(r=r, c=c):
                    row = pl.multiple_of(j * TM + r, HALO)
                    k = k_v[pl.ds(row, HALO + R), _tile(c)].astype(f32)[HALO - 8:]
                    acc = k[8:] * vec(z, TAP0, R, _tile(c))
                    for t in range(1, TAPS):
                        acc = acc + pltpu.roll(k, t, 0)[8:] * vec(z, TAP0 + t, R, _tile(c))
                    gated = acc * v_v[j, r:r + R, _tile(c)].astype(f32)
                    kv[j, r:r + R, _tile(c)] = gated
                    return _token(gated)
                short.append(('v', 18 * R // 8, short_conv))
        for i in range(BPS):
            for c in range(ND):
                def filter_dft(i=i, c=c):
                    h = jax.lax.dot_general(
                        _ld(fwd_u, z), _ld(filt_u, j * BPS + i, slice(c * 64, (c + 1) * 64)),
                        (((1,), (1,)), ((), ())), preferred_element_type=f32)
                    hs[j * BPS + i, 0:B, _tile(c)] = h[:B]
                    hs[j * BPS + i, B:N2, _tile(c)] = h[B:] - h[:B]
                    hs[j * BPS + i, N2:, _tile(c)] = h[B:] + h[:B]

                def input_dft(i=i, c=c):
                    x = jnp.dot(_ld(fwd_u, z), kv[z + j, i * B:(i + 1) * B, _tile(c)].astype(bf16),
                                preferred_element_type=f32)
                    xs[j * BPS + i, 0:B, _tile(c)] = x[:B] + x[B:]
                    xs[j * BPS + i, B:, _tile(c)] = x
                spectra += [('m', [N2], filter_dft), ('m', [N2], input_dft)]
        return short, spectra

    def convolve(j, nt):
        z = zero(j)
        last = j * BPS + BPS - 1
        xi = [z + jnp.where(d <= last, last - d, NB) for d in range(nt)]
        hi = [z + jnp.where(d <= last, d, NB) for d in range(nt)]
        terms = sum(nt - i for i in range(BPS))
        items = []
        for c in range(ND):
            for r in range(0, B, R):
                part = {}
                for k in range(3):
                    def products(r=r, c=c, k=k, part=part):
                        bins = slice(k * B + r, k * B + r + R)
                        acc, h = {}, []
                        for d in range(nt):
                            x = xs[xi[d], bins, _tile(c)]
                            h.append(hs[hi[d], bins, _tile(c)])
                            for i in range(BPS):
                                e = d - (BPS - 1 - i)
                                if e >= 0:
                                    acc[i] = x * h[e] if i not in acc else acc[i] + x * h[e]
                        if k < 2:
                            part[k] = acc
                            return _token(*acc.values())
                        pr, pi = carry[c, r:r + R, :], carry[c, B + r:B + r + R, :]
                        done = []
                        for i in range(BPS):
                            yr, yi = part[0][i] - acc[i], part[0][i] + part[1][i]
                            zr, zi = (yr - pi, yi + pr) if r < B // 2 else (yr + pi, yi - pr)
                            zb[i, c, 2 * r:2 * r + 2 * R, :] = (
                                jnp.concatenate([zr, zi], axis=0).astype(bf16))
                            done.append(zr)
                            pr, pi = yr, yi
                        carry[c, r:r + R, :] = pr
                        carry[c, B + r:B + r + R, :] = pi
                        return _token(*done)
                    items.append(('v', (2 * terms + 5) * (R // 8), products))
            for i in range(BPS):
                def inverse_dft(i=i, c=c):
                    g = jnp.concatenate([_ld(inv_u, z), _ld(inv_u, z + 1)], axis=1)
                    yb[0, i * B:(i + 1) * B, _tile(c)] = jnp.dot(
                        g, _ld(zb_u, z + i, c), preferred_element_type=f32)
                items.append(('m', [B, B], inverse_dft))
        return items

    def mixing(j):
        z = zero(j)
        early, late = [], []

        def mean(x):
            return jnp.sum(x, axis=-1, keepdims=True) * (1.0 / D)

        for r in range(0, TM, R):
            def q_stats(r=r):
                q = q_v[j, r:r + R, :].astype(f32)
                m = mean(q)
                qc = q - m
                rstd = jnp.broadcast_to(jax.lax.rsqrt(mean(qc * qc) + EPS), (R, 128))
                stat[0, r:r + R, :] = jnp.broadcast_to(m, (R, 128))
                stat[1, r:r + R, :] = rstd
                return _token(rstd)

            def residual(r=r):
                q = q_v[z + j, r:r + R, :].astype(f32)
                m, rstd = [jnp.concatenate([stat[z + i, r:r + R, :]] * ND, axis=1) for i in range(2)]
                h = (q - m) * rstd * vec(z, SCALE_A, R) + vec(z, SHIFT_A, R)
                y = yb[z, r:r + R, :] + kv[z + j, r:r + R, :] * vec(z, SKIP, R)
                x = q + vec(z, GATE_A, R) * (h * y)
                x2[j, r:r + R, :] = x
                xc = x - mean(x)
                h = xc * jax.lax.rsqrt(mean(xc * xc) + EPS) * vec(z, SCALE_B, R) + vec(z, SHIFT_B, R)
                for c in range(ND):
                    hb[c, r:r + R, :] = h[:, _tile(c)].astype(bf16)
                return _token(h[:, _tile(ND - 1)])
            early.append(('v', 6 * R // 8 * ND, q_stats))
            late.append(('v', 19 * R // 8 * ND, residual))
        return early, late

    def tied(z, tiles, ties):
        cols = []
        for kt, w in enumerate(tiles):
            for g in sorted(ties.get(kt, {})):
                keep = fwd_u[z, 0:8, :] != ones
                parts = [w[:8 * g], jnp.where(keep, w[8 * g:8 * g + 8], ties[kt][g]), w[8 * g + 8:]]
                w = jnp.concatenate([x for x in parts if x.shape[0]], axis=0)
            cols.append(w)
        return pltpu.bitcast(jnp.concatenate(cols, axis=1), bf16)

    def gate_up(j, first=False):
        dots, gate = [], {}
        z = zero(j)
        for i in range(NF):
            def gate_dot(ties, i=i):
                if first and i in GROUPS:
                    n = GROUPS.index(i)
                    _start(cp_down[n] if n < len(cp_down) else [])
                    _wait(cp_gu[n])
                g = 0.5 * jnp.dot(tied(z, [hb_u[z + c] for c in range(ND)], ties), _ld(w1_u, z + i),
                                  preferred_element_type=f32)
                gate[i] = g * jnp.tanh(g) + g

            def up_dot(ties, i=i):
                u = jnp.dot(tied(z, [hb_u[z + c] for c in range(ND)], ties), _ld(w3_u, z + i),
                            preferred_element_type=f32)
                act[i] = (gate[i] * u).astype(bf16)
            dots += [(ND, gate_dot), (ND, up_dot)]
        return dots

    def down(j, first=False, final=False):
        dots, total = [], {}
        z = zero(j)
        for c in range(ND):
            for k0 in range(0, NF, KD):
                def down_dot(ties, c=c, k0=k0):
                    if first and k0 == 0 and c == 0:
                        _wait(cp_down[0])
                        modulation(GATE_B)
                    if first and k0 == 0 and c == 3:
                        _start(step_inputs(3) + cp_rest)
                        _wait(cp_down[1])
                    tiles = [act_u[i if final else z + i] for i in range(k0, k0 + KD)]
                    o = jnp.dot(tied(z, tiles, ties), _ld(w2_u, z + c, slice(k0 * 64, (k0 + KD) * 64)),
                                preferred_element_type=f32)
                    total[c] = o if k0 == 0 else total[c] + o
                    if k0 + KD == NF:
                        out = x2[j, :, _tile(c)] + vec(z, GATE_B, TM, _tile(c)) * total[c]
                        ob[j, :, _tile(c)] = out.astype(bf16)
                        if final:
                            cp_out[NS - 1 + c].start()
                dots.append((KD, down_dot))
        return dots

    def warm_up(j, _):
        pl.when(j == 2)(lambda: _start(cp_gu[0]))
        pl.when(j == 0)(lambda: _start(step_inputs(1)))
        _wait(step_inputs(j))
        pl.when(j == 0)(lambda: _start(step_inputs(2) + cp_mod[0]))
        pl.when(j == 1)(lambda: _start(cp_mod[1]))
        _run(sum(transform(j), []))

    jax.lax.fori_loop(0, 3, warm_up, None)
    early, late = mixing(0)
    _run(convolve(0, BPS))
    _wait(cp_mod[0])
    for i in range(3):
        modulation(i)
    _run(early)
    _start(cp_gu[1] + cp_gu[2])
    _wait(cp_mod[1])
    modulation(SHIFT_B)
    modulation(SCALE_B)
    _run(late)

    _run_under(gate_up(0, first=True),
               [('after', 2 * GROUPS[-1] + 1, None), ('until', T_END, None)]
               + _mix(mixing(1)[0], convolve(1, 2 * BPS)))

    def step(j, nt, first=False):
        dots = down(j - 1, first)
        short, spectra = transform(jnp.minimum(j + 2, NS - 1))
        slack = 500 if first else 0
        items = [('until', T_POST, None)] + mixing(j)[1] + [('before', len(dots), None)]
        items += [('until', T_CONV + 3 * slack, None)] + convolve(j + 1, nt)
        if first:
            items.append(('v', 0, lambda: _wait(step_inputs(j + 2))))
        items += [('until', T_SHORT + slack, None)] + _mix(short, spectra[0::2])
        items += [('until', T_END, None)] + spectra[1::2] + mixing(j + 1)[0]
        _run_under(dots + gate_up(j), items)
        pltpu.make_async_copy(ob.at[j - 1], out_hbm.at[rows(j - 1)], sems.at[len(used) - 1]).start()

    step(1, 3 * BPS, first=True)
    _wait(cp_rest)
    jax.lax.fori_loop(2, NS - 1, lambda j, _: step(j, NB), None)

    dots = down(NS - 2)
    _run_under(dots + gate_up(NS - 1) + down(NS - 1, final=True),
               [('until', 12000, None)] + mixing(NS - 1)[1] + [('before', len(dots), None)]
               + [('after', len(dots), None), ('v', 0, lambda: cp_out[NS - 2].start())])
    _wait(cp_out)


@jax.jit
def pallas_adaLN_cond__ssm_conv_h3__glu_gated_swiglu__prompt_kernel(
        A_q, A_k, A_v, A_shift_k, A_ssm_k, A_ssm_D, B_x, B_w1, B_w3, B_w2, c, w_mod):
    del B_x
    fwd, inv = _dft_matrices()
    hbm = pl.BlockSpec(memory_space=pl.ANY)
    V = pltpu.VMEM
    out = pl.pallas_call(
        _kernel,
        out_shape=jax.ShapeDtypeStruct((S, D), bf16),
        in_specs=[hbm] * 13,
        out_specs=hbm,
        scratch_shapes=[
            V((NS, TM, D), bf16), V((HALO + S, D), bf16), V((NS, TM, D), bf16),
            V((TAPS, D), bf16), V((NB, D, B), bf16), V((D,), bf16),
            V((NF, D, 128), bf16), V((NF, D, 128), bf16), V((ND, FF, 128), bf16),
            V((1, D), bf16), V((D, 6 * D), bf16),
            V((1, N2, B), bf16), V((2, B, B), bf16),
            V((NB + 1, 3 * B, D), f32), V((NB + 1, 3 * B, D), f32),
            V((ND, N2, 128), f32), V((NS, TM, D), f32),
            V((BPS, ND, N2, 128), bf16), V((1, TM, D), f32),
            V((2, TM, 128), f32), V((NS, TM, D), f32),
            V((ND, TM, 128), bf16), V((NF, TM, 128), bf16), V((NS, TM, D), bf16),
            V((7 + TAPS, 8, D), f32),
            pltpu.SemaphoreType.DMA((7 + len(GROUPS),)),
            pltpu.SemaphoreType.DMA((4,)),
        ],
        compiler_params=pltpu.CompilerParams(vmem_limit_bytes=110 * 1024 * 1024),
    )(A_q.reshape(S, D), A_k.reshape(S, D), A_v.reshape(S, D), A_shift_k.T, A_ssm_k, A_ssm_D,
      B_w1, B_w3, B_w2, c, w_mod, fwd, inv)
    return out.reshape(1, S, D)
```

```python
import numpy as np
import jax
import jax.numpy as jnp
import jax.experimental.pallas as pl
import jax.experimental.pallas.tpu as pltpu

S, D, FF = 2048, 640, 1536
B = 128
NB = S // B
N2 = 2 * B
ND = D // 128
NF = FF // 128
TM = 256
NS = S // TM
BPS = TM // B
TAPS = 4
HALO = 16
R = 16
KD = 4
EPS = 1e-5
GROUPS = (0, 4, 8)

T_POST, T_CONV, T_SHORT, T_END = 10600, 2450, 1350, 300
OPERAND_LAG = 160

f32 = jnp.float32
bf16 = jnp.bfloat16
u32 = jnp.uint32


def _dft_matrices():
    freq = np.concatenate([np.arange(0, B, 2), np.arange(1, B, 2)])
    angle = 2.0 * np.pi * np.outer(freq + 0.5, np.arange(B)) / N2
    fwd = np.concatenate([np.cos(angle), -np.sin(angle)], axis=0)
    order = np.arange(N2).reshape(2, B // R, R).transpose(1, 0, 2).reshape(-1)
    inv = fwd[order].T / B
    inv = np.stack([inv[:, :B], inv[:, B:]])
    return fwd.astype(bf16), inv.astype(bf16)


def _ld(ref, *idx):
    return pltpu.bitcast(ref[idx], bf16)


def _token(*xs):
    tok = None
    for x in xs:
        x = pltpu.bitcast(x, u32)
        for r in range(0, x.shape[0], 8):
            tok = x[r:r + 8] if tok is None else tok | x[r:r + 8]
    return tok


def _tile(c):
    return slice(c * 128, (c + 1) * 128)


def _mix(a, b):
    keyed = [((i + 0.5) / len(t), n, i) for n, t in enumerate((a, b)) for i in range(len(t))]
    return [(a, b)[n][i] for _, n, i in sorted(keyed)]


def _start(copies):
    for cp in copies:
        cp.start()


def _wait(copies):
    for cp in copies:
        cp.wait()


def _run(items):
    for _, _, fn in items:
        if fn is not None:
            fn()


def _run_under(dots, items):
    total = (sum(nk * TM for nk, _ in dots) + sum(sum(c) for k, c, _ in items if k == 'm')) / 4
    free = [0, 0, 0, 0]
    unit = [0]

    def issue(lengths):
        starts = []
        for n in lengths:
            starts.append(free[unit[0] % 4])
            free[unit[0] % 4] += n
            unit[0] += 1
        return starts

    pos, now, end, left, held = 0, 0.0, 0, 0, []
    for n, (nk, dot) in enumerate(dots):
        while held and held[0][0] + OPERAND_LAG <= free[unit[0] % 4]:
            _, lengths, fn = held.pop(0)[1]
            fn()
            issue(lengths)
        starts = issue([TM] * nk)
        now = max(now, starts[0])
        ties = {}
        while pos < len(items):
            kind, c, fn = items[pos]
            if kind == 'm':
                held.append((now, items[pos]))
            elif kind == 'until':
                end, left = total - c, 0
                for k, cost, _ in items[pos + 1:]:
                    if k == 'until':
                        break
                    left += cost if k == 'v' else 0
            elif kind == 'after':
                if n < c:
                    break
            elif kind == 'v':
                due = now + c * max(end - now, 0) / max(left, 1)
                needed = any(k == 'before' and at == n + 1 for k, at, _ in items[pos:])
                if due >= starts[-1] + TM and not needed:
                    break
                tok = fn()
                now, left = due, left - c
                if tok is not None and due < starts[-1] + TM:
                    kt = max(t for t in range(nk) if t == 0 or starts[t] <= due)
                    g = int(min(max(due - starts[kt], 0) // 16, TM // 16 - 1))
                    slot = ties.setdefault(kt, {})
                    slot[g] = slot[g] | tok if g in slot else tok
            pos += 1
        dot(ties)
    _run([it for _, it in held] + items[pos:])


def _kernel(q_hbm, k_hbm, v_hbm, taps_hbm, filt_hbm, skip_hbm, w1_hbm, w3_hbm, w2_hbm, c_hbm,
            wmod_hbm, fwd_hbm, inv_hbm, out_hbm,
            q_v, k_v, v_v, taps_v, filt_v, skip_v, w1_v, w3_v, w2_v, c_v, wmod_v, fwd_v, inv_v,
            xs, hs, carry, kv, zb, yb, stat, x2, hb, act, ob, vecs, sems, step_sems):
    w1_u, w3_u, w2_u, filt_u, fwd_u, inv_u, kv_u, zb_u, hb_u, act_u = [
        r.bitcast(u32) for r in (w1_v, w3_v, w2_v, filt_v, fwd_v, inv_v, kv, zb, hb, act)]

    used = []

    def group(pairs):
        used.append(None)
        return [pltpu.make_async_copy(src, dst, sems.at[len(used) - 1]) for src, dst in pairs]

    def lanes(i):
        return pl.ds(i * 128 if isinstance(i, int) else pl.multiple_of(i * 128, 128), 128)

    def rows(j, skip=0):
        at = j * TM + skip
        return pl.ds(at if isinstance(j, int) else pl.multiple_of(at, HALO), TM)

    def input_pairs(j):
        pairs = [(filt_hbm.at[:, lanes(j * BPS + i)], filt_v.at[j * BPS + i]) for i in range(BPS)]
        return pairs + [(k_hbm.at[rows(j)], k_v.at[rows(j, HALO)]), (v_hbm.at[rows(j)], v_v.at[j]),
                        (q_hbm.at[rows(j)], q_v.at[j])]

    def step_inputs(j):
        return [pltpu.make_async_copy(src, dst, step_sems.at[j]) for src, dst in input_pairs(j)]

    mod = [(wmod_hbm.at[:, pl.ds(i * D, D)], wmod_v.at[:, pl.ds(i * D, D)]) for i in range(6)]
    w2 = [(w2_hbm.at[:, lanes(c)], w2_v.at[c]) for c in range(ND)]
    cp_small = group([(c_hbm, c_v), (taps_hbm, taps_v), (skip_hbm, skip_v),
                      (fwd_hbm, fwd_v.at[0]), (inv_hbm, inv_v)])
    cp_mod = [group([(wmod_hbm.at[:, pl.ds(lo * D, n * D)], wmod_v.at[:, pl.ds(lo * D, n * D)])])
              for lo, n in ((0, 3), (3, 2))]
    cp_gu = [group([(src.at[:, lanes(i)], dst.at[i])
                    for src, dst in ((w1_hbm, w1_v), (w3_hbm, w3_v)) for i in range(lo, hi)])
             for lo, hi in zip(GROUPS, GROUPS[1:] + (NF,))]
    cp_down = [group(w2[:3] + mod[5:]), group(w2[3:])]
    cp_rest = group(sum((input_pairs(j) for j in range(4, NS)), []))
    cp_out = group([(ob.at[j], out_hbm.at[rows(j)]) for j in range(NS - 1)]
                   + [(ob.at[NS - 1, :, lanes(c)], out_hbm.at[rows(NS - 1), lanes(c)]) for c in range(ND)])

    _start(cp_small + step_inputs(0))

    xs[NB] = jnp.zeros((3 * B, D), f32)
    hs[NB] = jnp.zeros((3 * B, D), f32)
    carry[...] = jnp.zeros((ND, N2, 128), f32)
    k_v[0:HALO, :] = jnp.zeros((HALO, D), bf16)
    _wait(cp_small)

    ones = jnp.uint32(0xFFFFFFFF)
    opaque = (fwd_u[0, 0, 0] == ones).astype(jnp.int32)

    def zero(j):
        return jnp.minimum(opaque, j + 1)

    SHIFT_A, SCALE_A, GATE_A, SHIFT_B, SCALE_B, GATE_B, TAP0, SKIP = 0, 1, 2, 3, 4, 5, 6, 6 + TAPS
    taps = taps_v[...].astype(f32)
    for t in range(TAPS):
        vecs[TAP0 + t] = jnp.broadcast_to(taps[t:t + 1], (8, D))
    vecs[SKIP] = jnp.broadcast_to(skip_v[...].astype(f32).reshape(1, D), (8, D))

    def modulation(i):
        c = c_v[...].astype(f32)
        s = jnp.broadcast_to(c * jax.nn.sigmoid(c), (16, D)).astype(bf16)
        m = jnp.dot(s, wmod_v[:, i * D:(i + 1) * D], preferred_element_type=f32)[0:8]
        vecs[i] = 1.0 + m if i in (SCALE_A, SCALE_B) else m

    def vec(z, i, n, cols=slice(None)):
        return jnp.concatenate([vecs[z + i, :, cols]] * (n // 8), axis=0)

    def transform(j):
        z = zero(j)
        short, spectra = [], []
        for r in range(0, TM, R):
            for c in range(ND):
                def short_conv(r=r, c=c):
                    row = pl.multiple_of(j * TM + r, HALO)
                    k = k_v[pl.ds(row, HALO + R), _tile(c)].astype(f32)[HALO - 8:]
                    acc = k[8:] * vec(z, TAP0, R, _tile(c))
                    for t in range(1, TAPS):
                        acc = acc + pltpu.roll(k, t, 0)[8:] * vec(z, TAP0 + t, R, _tile(c))
                    gated = acc * v_v[j, r:r + R, _tile(c)].astype(f32)
                    kv[j * ND + c, r:r + R, :] = gated.astype(bf16)
                    return _token(gated)
                short.append(('v', 18 * R // 8, short_conv))
        for i in range(BPS):
            for c in range(ND):
                def filter_dft(i=i, c=c):
                    h = jax.lax.dot_general(
                        _ld(fwd_u, z), _ld(filt_u, j * BPS + i, slice(c * 64, (c + 1) * 64)),
                        (((1,), (1,)), ((), ())), preferred_element_type=f32)
                    hs[j * BPS + i, 0:B, _tile(c)] = h[:B]
                    hs[j * BPS + i, B:N2, _tile(c)] = h[B:] - h[:B]
                    hs[j * BPS + i, N2:, _tile(c)] = h[B:] + h[:B]

                def input_dft(i=i, c=c):
                    x = jnp.dot(_ld(fwd_u, z), _ld(kv_u, z + j * ND + c, slice(i * B // 2, (i + 1) * B // 2)),
                                preferred_element_type=f32)
                    xs[j * BPS + i, 0:B, _tile(c)] = x[:B] + x[B:]
                    xs[j * BPS + i, B:, _tile(c)] = x
                spectra += [('m', [N2], filter_dft), ('m', [N2], input_dft)]
        return short, spectra

    def convolve(j, nt):
        z = zero(j)
        last = j * BPS + BPS - 1
        xi = [z + jnp.where(d <= last, last - d, NB) for d in range(nt)]
        hi = [z + jnp.where(d <= last, d, NB) for d in range(nt)]
        terms = sum(nt - i for i in range(BPS))
        items = []
        for c in range(ND):
            for r in range(0, B, R):
                part = {}
                for k in range(3):
                    def products(r=r, c=c, k=k, part=part):
                        bins = slice(k * B + r, k * B + r + R)
                        acc, h = {}, []
                        for d in range(nt):
                            x = xs[xi[d], bins, _tile(c)]
                            h.append(hs[hi[d], bins, _tile(c)])
                            for i in range(BPS):
                                e = d - (BPS - 1 - i)
                                if e >= 0:
                                    acc[i] = x * h[e] if i not in acc else acc[i] + x * h[e]
                        if k < 2:
                            part[k] = acc
                            return _token(*acc.values())
                        pr, pi = carry[c, r:r + R, :], carry[c, B + r:B + r + R, :]
                        done = []
                        for i in range(BPS):
                            yr, yi = part[0][i] - acc[i], part[0][i] + part[1][i]
                            zr, zi = (yr - pi, yi + pr) if r < B // 2 else (yr + pi, yi - pr)
                            zb[i, c, 2 * r:2 * r + 2 * R, :] = (
                                jnp.concatenate([zr, zi], axis=0).astype(bf16))
                            done.append(zr)
                            pr, pi = yr, yi
                        carry[c, r:r + R, :] = pr
                        carry[c, B + r:B + r + R, :] = pi
                        return _token(*done)
                    items.append(('v', (2 * terms + 5) * (R // 8), products))
            for i in range(BPS):
                def inverse_dft(i=i, c=c):
                    g = jnp.concatenate([_ld(inv_u, z), _ld(inv_u, z + 1)], axis=1)
                    yb[0, i * B:(i + 1) * B, _tile(c)] = jnp.dot(
                        g, _ld(zb_u, z + i, c), preferred_element_type=f32)
                items.append(('m', [B, B], inverse_dft))
        return items

    def mixing(j):
        z = zero(j)
        early, late = [], []

        def mean(x):
            return jnp.sum(x, axis=-1, keepdims=True) * (1.0 / D)

        for r in range(0, TM, R):
            def q_stats(r=r):
                q = q_v[j, r:r + R, :].astype(f32)
                m = mean(q)
                qc = q - m
                rstd = jnp.broadcast_to(jax.lax.rsqrt(mean(qc * qc) + EPS), (R, 128))
                stat[0, r:r + R, :] = jnp.broadcast_to(m, (R, 128))
                stat[1, r:r + R, :] = rstd
                return _token(rstd)

            def residual(r=r):
                q = q_v[z + j, r:r + R, :].astype(f32)
                m, rstd = [jnp.concatenate([stat[z + i, r:r + R, :]] * ND, axis=1) for i in range(2)]
                h = (q - m) * rstd * vec(z, SCALE_A, R) + vec(z, SHIFT_A, R)
                gated = jnp.concatenate([kv[z + j * ND + c, r:r + R, :].astype(f32)
                                         for c in range(ND)], axis=1)
                y = yb[z, r:r + R, :] + gated * vec(z, SKIP, R)
                x = q + vec(z, GATE_A, R) * (h * y)
                x2[j, r:r + R, :] = x
                xc = x - mean(x)
                h = xc * jax.lax.rsqrt(mean(xc * xc) + EPS) * vec(z, SCALE_B, R) + vec(z, SHIFT_B, R)
                for c in range(ND):
                    hb[c, r:r + R, :] = h[:, _tile(c)].astype(bf16)
                return _token(h[:, _tile(ND - 1)])
            early.append(('v', 6 * R // 8 * ND, q_stats))
            late.append(('v', 19 * R // 8 * ND, residual))
        return early, late

    def tied(z, tiles, ties):
        cols = []
        for kt, w in enumerate(tiles):
            for g in sorted(ties.get(kt, {})):
                keep = fwd_u[z, 0:8, :] != ones
                parts = [w[:8 * g], jnp.where(keep, w[8 * g:8 * g + 8], ties[kt][g]), w[8 * g + 8:]]
                w = jnp.concatenate([x for x in parts if x.shape[0]], axis=0)
            cols.append(w)
        return pltpu.bitcast(jnp.concatenate(cols, axis=1), bf16)

    def gate_up(j, first=False):
        dots, gate = [], {}
        z = zero(j)
        for i in range(NF):
            def gate_dot(ties, i=i):
                if first and i in GROUPS:
                    n = GROUPS.index(i)
                    _start(cp_down[n] if n < len(cp_down) else [])
                    _wait(cp_gu[n])
                g = 0.5 * jnp.dot(tied(z, [hb_u[z + c] for c in range(ND)], ties), _ld(w1_u, z + i),
                                  preferred_element_type=f32)
                gate[i] = g * jnp.tanh(g) + g

            def up_dot(ties, i=i):
                u = jnp.dot(tied(z, [hb_u[z + c] for c in range(ND)], ties), _ld(w3_u, z + i),
                            preferred_element_type=f32)
                act[i] = (gate[i] * u).astype(bf16)
            dots += [(ND, gate_dot), (ND, up_dot)]
        return dots

    def down(j, first=False, final=False):
        dots, total = [], {}
        z = zero(j)
        for c in range(ND):
            for k0 in range(0, NF, KD):
                def down_dot(ties, c=c, k0=k0):
                    if first and k0 == 0 and c == 0:
                        _wait(cp_down[0])
                        modulation(GATE_B)
                    if first and k0 == 0 and c == 3:
                        _start(step_inputs(3) + cp_rest)
                        _wait(cp_down[1])
                    tiles = [act_u[i if final else z + i] for i in range(k0, k0 + KD)]
                    o = jnp.dot(tied(z, tiles, ties), _ld(w2_u, z + c, slice(k0 * 64, (k0 + KD) * 64)),
                                preferred_element_type=f32)
                    total[c] = o if k0 == 0 else total[c] + o
                    if k0 + KD == NF:
                        out = x2[j, :, _tile(c)] + vec(z, GATE_B, TM, _tile(c)) * total[c]
                        ob[j, :, _tile(c)] = out.astype(bf16)
                        if final:
                            cp_out[NS - 1 + c].start()
                dots.append((KD, down_dot))
        return dots

    def warm_up(j, _):
        pl.when(j == 2)(lambda: _start(cp_gu[0]))
        pl.when(j == 0)(lambda: _start(step_inputs(1)))
        _wait(step_inputs(j))
        pl.when(j == 0)(lambda: _start(step_inputs(2) + cp_mod[0]))
        pl.when(j == 1)(lambda: _start(cp_mod[1]))
        _run(sum(transform(j), []))

    jax.lax.fori_loop(0, 3, warm_up, None)
    early, late = mixing(0)
    _run(convolve(0, BPS))
    _wait(cp_mod[0])
    for i in range(3):
        modulation(i)
    _run(early)
    _start(cp_gu[1] + cp_gu[2])
    _wait(cp_mod[1])
    modulation(SHIFT_B)
    modulation(SCALE_B)
    _run(late)

    _run_under(gate_up(0, first=True),
               [('after', 2 * GROUPS[-1] + 1, None), ('until', T_END, None)]
               + _mix(mixing(1)[0], convolve(1, 2 * BPS)))

    def step(j, nt, first=False):
        dots = down(j - 1, first)
        short, spectra = transform(jnp.minimum(j + 2, NS - 1))
        slack = 500 if first else 0
        items = [('until', T_POST, None)] + mixing(j)[1] + [('before', len(dots), None)]
        items += [('until', T_CONV + 3 * slack, None)] + convolve(j + 1, nt)
        if first:
            items.append(('v', 0, lambda: _wait(step_inputs(j + 2))))
        items += [('until', T_SHORT + slack, None)] + _mix(short, spectra[0::2])
        items += [('until', T_END, None)] + spectra[1::2] + mixing(j + 1)[0]
        _run_under(dots + gate_up(j), items)
        pltpu.make_async_copy(ob.at[j - 1], out_hbm.at[rows(j - 1)], sems.at[len(used) - 1]).start()

    step(1, 3 * BPS, first=True)
    _wait(cp_rest)
    jax.lax.fori_loop(2, NS - 1, lambda j, _: step(j, NB), None)

    dots = down(NS - 2)
    _run_under(dots + gate_up(NS - 1) + down(NS - 1, final=True),
               [('until', 12000, None)] + mixing(NS - 1)[1] + [('before', len(dots), None)]
               + [('after', len(dots), None), ('v', 0, lambda: cp_out[NS - 2].start())])
    _wait(cp_out)


@jax.jit
def pallas_adaLN_cond__ssm_conv_h3__glu_gated_swiglu__prompt_kernel(
        A_q, A_k, A_v, A_shift_k, A_ssm_k, A_ssm_D, B_x, B_w1, B_w3, B_w2, c, w_mod):
    del B_x
    fwd, inv = _dft_matrices()
    hbm = pl.BlockSpec(memory_space=pl.ANY)
    V = pltpu.VMEM
    out = pl.pallas_call(
        _kernel,
        out_shape=jax.ShapeDtypeStruct((S, D), bf16),
        in_specs=[hbm] * 13,
        out_specs=hbm,
        scratch_shapes=[
            V((NS, TM, D), bf16), V((HALO + S, D), bf16), V((NS, TM, D), bf16),
            V((TAPS, D), bf16), V((NB, D, B), bf16), V((D,), bf16),
            V((NF, D, 128), bf16), V((NF, D, 128), bf16), V((ND, FF, 128), bf16),
            V((1, D), bf16), V((D, 6 * D), bf16),
            V((1, N2, B), bf16), V((2, B, B), bf16),
            V((NB + 1, 3 * B, D), f32), V((NB + 1, 3 * B, D), f32),
            V((ND, N2, 128), f32), V((NS * ND, TM, 128), bf16),
            V((BPS, ND, N2, 128), bf16), V((1, TM, D), f32),
            V((2, TM, 128), f32), V((NS, TM, D), f32),
            V((ND, TM, 128), bf16), V((NF, TM, 128), bf16), V((NS, TM, D), bf16),
            V((7 + TAPS, 8, D), f32),
            pltpu.SemaphoreType.DMA((7 + len(GROUPS),)),
            pltpu.SemaphoreType.DMA((4,)),
        ],
        compiler_params=pltpu.CompilerParams(vmem_limit_bytes=110 * 1024 * 1024),
    )(A_q.reshape(S, D), A_k.reshape(S, D), A_v.reshape(S, D), A_shift_k.T, A_ssm_k, A_ssm_D,
      B_w1, B_w3, B_w2, c, w_mod, fwd, inv)
    return out.reshape(1, S, D)
```
